```python
import os as _os
_os.environ.setdefault('JAX_PLATFORMS', 'cpu')
import jax
import jax.numpy as jnp

def _softmax(x, axis=-1):
    return jax.nn.softmax(x, axis=axis)

def _gelu(x):
    return jax.nn.gelu(x, approximate=True)

def _silu(x):
    return jax.nn.silu(x)

def _sigmoid(x):
    return jax.nn.sigmoid(x)

def _layernorm(x, axis=-1, eps=1e-05):
    m = jnp.mean(x, axis=axis, keepdims=True)
    v = jnp.var(x, axis=axis, keepdims=True)
    return (x - m) / jnp.sqrt(v + eps)

def _scatter_add(tgt, idx, src, axis=0):
    return tgt.at[idx].add(src)

def _segment_sum(src, seg, n):
    return jax.ops.segment_sum(src, seg, n)

class _Rng:

    def __init__(self, key):
        self._k = key

    def _next(self):
        self._k, sub = jax.random.split(self._k)
        return sub

    def normal(self, shape):
        return jax.random.normal(self._next(), shape, dtype=jnp.bfloat16)

    def randint(self, lo, hi, shape):
        return jax.random.randint(self._next(), shape, lo, hi, dtype=jnp.int32)

    def uniform(self, shape, lo=0.0, hi=1.0):
        return jax.random.uniform(self._next(), shape, jnp.bfloat16, lo, hi)

    def permutation(self, n):
        return jax.random.permutation(self._next(), n)
kernel_name = 'standalone__window_attn_twins__vision'

def setup_inputs():
    _rng = _Rng(jax.random.key(int.from_bytes(__import__("os").urandom(4), "little")))
    _w = lambda a: (lambda t: t.astype(jnp.bfloat16) if jnp.issubdtype(t.dtype, jnp.floating) else t)(jnp.asarray(a))
    H = W = 384 // 8 * 8
    C = 96
    return {'x': _w((lambda *s: _rng.normal(s) * 0.4)(1, H, W, C)), 'wq': _w((lambda *s: _rng.normal(s) * 0.4)(C, C)), 'wkv': _w((lambda *s: _rng.normal(s) * 0.4)(C, 2 * C)), 'wo': _w((lambda *s: _rng.normal(s) * 0.05)(C, C))}

def reference(x, wq, wkv, wo):
    B, H, W, C = x.shape
    win = 8
    nh, nw = (H // win, W // win)
    xs = x.reshape(B, nh, win, nw, win, C).mean(axis=(2, 4)).reshape(B, nh * nw, C)
    q = x.reshape(B, H * W, C) @ wq
    kv = xs @ wkv
    k, v = (kv[..., :C].copy(), kv[..., C:].copy())
    scale = C ** (-0.5)
    p = _softmax(jnp.einsum('bqc,bkc->bqk', q, k) * scale, axis=-1)
    o = jnp.einsum('bqk,bkc->bqc', p, v) @ wo
    return o.reshape(B, H, W, C)
```

```python
import functools
import math

import jax
import jax.numpy as jnp
import jax.experimental.pallas as pl
import jax.experimental.pallas.tpu as pltpu

WIN = 8
ROWS_PER_STEP = 4


def _kernel(x_ref, wq_ref, wkv_ref, wo_ref, o_ref, xs_ref, at_ref, bt_ref, *, H, W, C):
    nh, nw = H // WIN, W // WIN
    step = pl.program_id(0)
    f32, bf16 = jnp.float32, jnp.bfloat16

    @pl.when(step == 0)
    def _prologue():
        jj = jax.lax.broadcasted_iota(jnp.int32, (nw, W), 0)
        ww = jax.lax.broadcasted_iota(jnp.int32, (nw, W), 1)
        pool = jnp.where((ww >= jj * WIN) & (ww < (jj + 1) * WIN), 1.0, 0.0).astype(bf16)

        def body(i, carry):
            blk = x_ref[pl.ds(i * WIN, WIN)].astype(f32)
            ssum = jnp.sum(blk, axis=0)
            hi = ssum.astype(bf16)
            lo = (ssum - hi.astype(f32)).astype(bf16)
            dn = (((1,), (1,)), ((), ()))
            r = jax.lax.dot_general(pool, hi, dn, preferred_element_type=f32)
            r = r + jax.lax.dot_general(pool, lo, dn, preferred_element_type=f32)
            xs_ref[pl.ds(pl.multiple_of(i * nw, 8), nw), :] = r * (1.0 / (WIN * WIN))
            return carry

        jax.lax.fori_loop(0, nh, body, 0)
        xs = xs_ref[...].astype(bf16)
        kv = jnp.dot(xs, wkv_ref[...], preferred_element_type=f32)
        k = kv[:, :C].astype(bf16)
        v = kv[:, C:].astype(bf16)
        dn = (((1,), (1,)), ((), ()))
        at = jax.lax.dot_general(k, wq_ref[...], dn, preferred_element_type=f32)
        at_ref[...] = (at * (C ** -0.5 * math.log2(math.e))).astype(bf16)
        b = jnp.dot(v, wo_ref[...], preferred_element_type=f32)
        bt_ref[...] = b.T.astype(bf16)

    for r in range(ROWS_PER_STEP):
        xt = x_ref[step * ROWS_PER_STEP + r]
        st = jnp.dot(at_ref[...], xt, preferred_element_type=f32)
        m = jnp.max(st, axis=0, keepdims=True)
        p = jnp.exp2(st - m)
        l = jnp.sum(p, axis=0, keepdims=True)
        ot = jnp.dot(bt_ref[...], p.astype(bf16), preferred_element_type=f32)
        o_ref[r] = (ot * (1.0 / l)).astype(o_ref.dtype)


@jax.jit
def pallas_standalone__window_attn_twins__vision_kernel(x, wq, wkv, wo):
    B, H, W, C = x.shape
    assert B == 1
    nk = (H // WIN) * (W // WIN)
    xt = jnp.transpose(x, (0, 1, 3, 2)).reshape(H, C, W)
    out = pl.pallas_call(
        functools.partial(_kernel, H=H, W=W, C=C),
        grid=(H // ROWS_PER_STEP,),
        in_specs=[
            pl.BlockSpec((H, C, W), lambda i: (0, 0, 0), pipeline_mode=pl.Buffered(1)),
            pl.BlockSpec((C, C), lambda i: (0, 0)),
            pl.BlockSpec((C, 2 * C), lambda i: (0, 0)),
            pl.BlockSpec((C, C), lambda i: (0, 0)),
        ],
        out_specs=pl.BlockSpec((ROWS_PER_STEP, C, W), lambda i: (i, 0, 0)),
        out_shape=jax.ShapeDtypeStruct((H, C, W), x.dtype),
        scratch_shapes=[
            pltpu.VMEM((nk, C), jnp.float32),
            pltpu.VMEM((nk, C), jnp.bfloat16),
            pltpu.VMEM((C, nk), jnp.bfloat16),
        ],
        compiler_params=pltpu.CompilerParams(
            dimension_semantics=("arbitrary",),
            vmem_limit_bytes=100 * 1024 * 1024,
        ),
    )(xt, wq, wkv, wo)
    return jnp.transpose(out.reshape(1, H, C, W), (0, 1, 3, 2))
```

```python
import functools
import math

import jax, jax.numpy as jnp
import jax.experimental.pallas as pl
import jax.experimental.pallas.tpu as pltpu

WIN = 8
f32, bf16, u32 = jnp.float32, jnp.bfloat16, jnp.uint32
LANE = 128

def _attend(x_vm, row0, R, at_tile, bt_tile, nkt, sr, zero, o_ref, state, *, W, C, TQ, skew, pb):
    NB = len(sr)
    tpg = TQ // LANE
    G = R * W // TQ
    wt = W // LANE
    never = zero != 0
    M = {}; MF = {}; L = {}; ACC = {}; XQ = {}; AL = {}

    def loc(t):
        r, c = divmod(t, wt)
        return r, slice(c * LANE, (c + 1) * LANE)

    def qk(g, j):
        if g not in XQ:
            XQ[g] = jnp.concatenate([x_vm[row0 + loc(g * tpg + t)[0], :, loc(g * tpg + t)[1]] for t in range(tpg)], axis=1)
        s = jnp.dot(pltpu.bitcast(at_tile(j), bf16), XQ[g], preferred_element_type=f32)
        sr[g % NB][0, j * LANE:(j + 1) * LANE, :] = s
        mj = jnp.max(s.reshape(LANE // 8, 8, TQ), axis=0)
        M[g] = mj if j == 0 else jnp.maximum(M[g], mj)
        if j == nkt - 1:
            MF[g] = jnp.max(M[g], axis=0, keepdims=True)

    def pv(g, uj):
        u, j = divmod(uj, nkt)
        t = g * tpg + u
        r, cs = loc(t)
        us = slice(u * LANE, (u + 1) * LANE)
        if j == 0:
            m = jnp.broadcast_to(MF[g][:, us], (8, LANE))
            if state is not None:
                m_ref, l_ref, acc_ref = state
                m_old = m_ref[t]
                m = jnp.maximum(m, m_old)
                alpha = jnp.exp2(m_old - m)
                m_ref[t] = m
                L[t] = l_ref[t] * alpha
                AL[t] = alpha
            else:
                L[t] = zero
            M[('t', t)] = m
        m = M[('t', t)]
        p = jnp.exp2(sr[g % NB][0, j * LANE:(j + 1) * LANE, us].reshape(LANE // 8, 8, LANE) - m[None])
        l = L[t] + jnp.sum(p, axis=0)
        L[t] = l
        p = p.reshape(LANE, LANE)
        p = jnp.concatenate([jnp.where(never, l, p[0:8, :]), p[8:, :]], axis=0)
        o = jnp.dot(pltpu.bitcast(bt_tile(j), bf16), p.astype(bf16), preferred_element_type=f32)
        ACC[t] = o if t not in ACC else o + ACC[t]
        if j == nkt - 1:
            acc = ACC[t]
            if state is not None:
                m_ref, l_ref, acc_ref = state
                acc = acc + (acc_ref[t].reshape(C // 8, 8, LANE) * AL[t][None]).reshape(C, LANE)
                acc_ref[t] = acc
                l_ref[t] = l
            lt = jnp.sum(l, axis=0, keepdims=True)
            o_ref[r, :, cs] = (acc * (1.0 / lt)).astype(o_ref.dtype)

    qev = [('qk', g, j) for g in range(G) for j in range(nkt)]
    pev = [('pv', g, uj) for g in range(G) for uj in range(tpg * nkt)]
    events = []
    for i, e in enumerate(qev):
        events.append((i * tpg, 0, i, e))
    for i, e in enumerate(pev):
        events.append((nkt * tpg + skew + (i // pb) * pb, 1, i, e))
    events.sort()
    for _, _, _, (kind, g, j) in events:
        (qk if kind == 'qk' else pv)(g, j)


def _kernel(x_hbm, wq_ref, wkv_ref, wo_ref, o_ref, x_vm, sems, at_ref, bt_ref, zi_ref, m_ref, l_ref, acc_ref, *sr,
            H, W, C, R, TQ, skew, pb, skew_e, dma_mode):
    step = pl.program_id(0)
    NS, SK = bt_ref.shape[0], bt_ref.shape[2]
    NK = NS * SK
    nw = W // WIN
    cps = SK // nw
    rps = cps * WIN
    kts = SK // LANE

    def copy(s):
        return pltpu.make_async_copy(x_hbm.at[pl.ds(s * rps, rps)], x_vm.at[pl.ds(s * rps, rps)], sems.at[s])

    def opaque_zero():
        zd = zi_ref[0]
        return sum(s_[zd, NK:NK + 8, 0:LANE] for s_ in sr)

    @pl.when(step == 0)
    def _early():
        if dma_mode == 0:
            for s in range(NS): copy(s).start()
        else:
            copy(0).start()
        zi_ref[0] = 0
        for s_ in sr: s_[0, NK:NK + 8, :] = jnp.zeros((8, TQ), f32)
        m_ref[...] = jnp.full(m_ref.shape, -jnp.inf, f32)
        l_ref[...] = jnp.zeros(l_ref.shape, f32)
        acc_ref[...] = jnp.zeros(acc_ref.shape, f32)

        def stage(s, carry):
            copy(s).wait()
            if dma_mode == 1:
                @pl.when(s + 1 < NS)
                def _():
                    copy(s + 1).start()
            jj = jax.lax.broadcasted_iota(jnp.int32, (nw, W), 0)
            ww = jax.lax.broadcasted_iota(jnp.int32, (nw, W), 1)
            pool = jnp.where((ww >= jj * WIN) & (ww < (jj + 1) * WIN), 1.0, 0.0).astype(bf16)
            nt = (((1,), (1,)), ((), ()))
            xs = []
            for i in range(cps):
                blk = x_vm[pl.ds(s * rps + i * WIN, WIN)].astype(f32)
                ssum = jnp.sum(blk, axis=0)
                hi = ssum.astype(bf16)
                lo = (ssum - hi.astype(f32)).astype(bf16)
                r = jax.lax.dot_general(pool, hi, nt, preferred_element_type=f32)
                r = r + jax.lax.dot_general(pool, lo, nt, preferred_element_type=f32)
                xs.append((r * (1.0 / (WIN * WIN))).astype(bf16))
            xs = jnp.concatenate(xs, axis=0)
            k = jnp.dot(xs, wkv_ref[:, :C], preferred_element_type=f32).astype(bf16)
            v = jnp.dot(xs, wkv_ref[:, C:], preferred_element_type=f32).astype(bf16)
            at = jax.lax.dot_general(k, wq_ref[...], nt, preferred_element_type=f32)
            at_ref[s] = pltpu.bitcast((at * (C ** -0.5 * math.log2(math.e))).astype(bf16), u32)
            bt = jax.lax.dot_general(wo_ref[...].T, v, nt, preferred_element_type=f32)
            bt_ref[s] = pltpu.bitcast(bt.astype(bf16), u32)
            _attend(x_vm, 0, R,
                    lambda j: at_ref[s, j * 64:(j + 1) * 64, :],
                    lambda j: bt_ref[s, :, j * LANE:(j + 1) * LANE],
                    kts, sr, opaque_zero(), o_ref, (m_ref, l_ref, acc_ref), W=W, C=C, TQ=TQ, skew=skew_e, pb=pb)
            return carry
        jax.lax.fori_loop(0, NS, stage, 0)

    @pl.when(step > 0)
    def _main():
        _attend(x_vm, step * R, R,
                lambda j: at_ref[j // kts, (j % kts) * 64:(j % kts + 1) * 64, :],
                lambda j: bt_ref[j // kts, :, (j % kts) * LANE:(j % kts + 1) * LANE],
                NS * kts, sr[:3], opaque_zero(), o_ref, None, W=W, C=C, TQ=TQ, skew=skew, pb=pb)


@jax.jit
def pallas_standalone__window_attn_twins__vision_kernel(x, wq, wkv, wo):
    B, H, W, C = x.shape
    assert B == 1
    R, TQ, NB, SK = 16, 512, 4, 384
    nk = (H // WIN) * (W // WIN)
    NS = nk // SK
    ntile = R * W // LANE
    xt = jnp.transpose(x, (0, 1, 3, 2)).reshape(H, C, W)
    out = pl.pallas_call(
        functools.partial(_kernel, H=H, W=W, C=C, R=R, TQ=TQ, skew=12, pb=4, skew_e=12, dma_mode=0),
        grid=(H // R,),
        in_specs=[
            pl.BlockSpec(memory_space=pl.ANY),
            pl.BlockSpec((C, C), lambda i: (0, 0)),
            pl.BlockSpec((C, 2 * C), lambda i: (0, 0)),
            pl.BlockSpec((C, C), lambda i: (0, 0)),
        ],
        out_specs=pl.BlockSpec((R, C, W), lambda i: (i, 0, 0)),
        out_shape=jax.ShapeDtypeStruct((H, C, W), x.dtype),
        scratch_shapes=[
            pltpu.VMEM((H, C, W), bf16), pltpu.SemaphoreType.DMA((NS,)),
            pltpu.VMEM((NS, SK // 2, C), u32), pltpu.VMEM((NS, C // 2, SK), u32),
            pltpu.SMEM((1,), jnp.int32),
            pltpu.VMEM((ntile, 8, LANE), f32), pltpu.VMEM((ntile, 8, LANE), f32), pltpu.VMEM((ntile, C, LANE), f32),
        ] + [pltpu.VMEM((1, nk + 8, TQ), f32)] * NB,
        compiler_params=pltpu.CompilerParams(dimension_semantics=("arbitrary",), vmem_limit_bytes=100 * 1024 * 1024),
    )(xt, wq, wkv, wo)
    return jnp.transpose(out.reshape(1, H, C, W), (0, 1, 3, 2))
```

```python
import functools
import math

import jax
import jax.numpy as jnp
import jax.experimental.pallas as pl
import jax.experimental.pallas.tpu as pltpu

f32, bf16, u32 = jnp.float32, jnp.bfloat16, jnp.uint32
WIN = 8
LANE = 128
NT = (((1,), (1,)), ((), ()))

R = 16
RE = 32
SK = 384
TQ = 512
NR = 2
RO = 3
CFG = dict(skew=16, gap=12, off=8, dly=8, gap2=4, skew_e=6, off2=6, pb_pos=10, late=8)


def _colmax(s):
    return jnp.max(s.reshape(s.shape[0] // 8, 8, s.shape[1]), axis=0)


def _allmax(m):
    return jnp.broadcast_to(jnp.max(m, axis=0, keepdims=True), m.shape)


def _pv_unit(sv, m, l, acc, bt, never):
    p = jnp.exp2(sv.reshape(LANE // 8, 8, LANE) - m[None])
    l = l + jnp.sum(p, axis=0)
    p = p.reshape(LANE, LANE)
    p = jnp.concatenate([jnp.where(never, l, p[0:8, :]), p[8:, :]], axis=0)
    o = jnp.dot(pltpu.bitcast(bt, bf16), p.astype(bf16), preferred_element_type=f32)
    return l, (o if acc is None else o + acc)


def _interleave(main, extra):
    extra = sorted(extra, key=lambda e: e[:2])
    for i, fn in enumerate(main):
        while extra and extra[0][0] <= i:
            extra.pop(0)[2]()
        fn()
    for e in extra:
        e[2]()


def _kernel(x_hbm, wq_hbm, wkv_hbm, wo_hbm, o_hbm,
            o_vm, osem, x_vm, xsems, wq_ref, wkv_ref, wo_ref, wsem, at_ref, bt_ref, wf_ref, xs_ref,
            zi_ref, mp_ref, m_ref, l_ref, acc_ref, *sr,
            H, W, C, skew, gap, off, dly, gap2, skew_e, off2, pb_pos, late):
    step = pl.program_id(0)
    NS = bt_ref.shape[0]
    NK = NS * SK
    PK = 2 * W // WIN
    rpp = 2 * WIN
    npair = SK // PK
    kts = SK // LANE
    wt = W // LANE
    tpg = TQ // LANE
    NB = len(sr)
    nte = RE * wt
    nev = RE // NR

    def xcopy(p):
        rows = pl.ds(p * rpp, rpp)
        return pltpu.make_async_copy(x_hbm.at[rows], x_vm.at[rows], xsems.at[p])

    def ocopy(r0, n):
        rows = pl.ds(r0, n)
        return pltpu.make_async_copy(o_vm.at[rows], o_hbm.at[rows], osem.at[0])

    def opaque_zero():
        zd = zi_ref[0]
        return sum(s_[zd, NK:NK + 8, 0:LANE] for s_ in sr)

    def x_tile(row0, t):
        return x_vm[row0 + t // wt, :, (t % wt) * LANE:(t % wt + 1) * LANE]

    def normalise(row0, t, acc, l):
        r, c = divmod(t, wt)
        lt = jnp.sum(l, axis=0, keepdims=True)
        o_vm[row0 + r, :, c * LANE:(c + 1) * LANE] = (acc * (1.0 / lt)).astype(o_vm.dtype)

    def eloc(t):
        b, q = t % NB, t // NB
        return sr[b], (q // tpg) * SK, (q % tpg) * LANE

    def pool_events(p, pos0, gap_, prow=None):
        kpt = LANE // WIN
        jj = jax.lax.broadcasted_iota(jnp.int32, (kpt, LANE), 0)
        ww = jax.lax.broadcasted_iota(jnp.int32, (kpt, LANE), 1)
        pool = jnp.where((ww >= jj * WIN) & (ww < (jj + 1) * WIN), 1.0 / (WIN * WIN), 0.0).astype(bf16)
        prow = p if prow is None else prow
        means = {}

        def piece(k):
            def run():
                i, c = divmod(k, wt)
                blk = x_vm[pl.ds(prow * rpp + i * WIN, WIN), :, c * LANE:(c + 1) * LANE]
                ssum = jnp.sum(blk.astype(f32), axis=0)
                hi = ssum.astype(bf16)
                lo = (ssum - hi.astype(f32)).astype(bf16)
                r = jax.lax.dot_general(pool, hi, NT, preferred_element_type=f32)
                r = jax.lax.dot_general(pool, lo, NT, preferred_element_type=f32) + r
                means[k] = r.astype(bf16)
            return run

        def proj():
            xs = jnp.concatenate([means[k] for k in range(2 * wt)], axis=0)
            xs_ref[prow] = pltpu.bitcast(xs, u32)
            at = jnp.dot(xs, pltpu.bitcast(wf_ref[0], bf16), preferred_element_type=f32)
            at_ref[p] = pltpu.bitcast(at.astype(bf16), u32)

        ev = [(pos0 + k * gap_, 0, piece(k)) for k in range(2 * wt)]
        ev.append((pos0 + (2 * wt - 1) * gap_ + (dly if gap_ else 0), 1, proj))
        return ev

    def proj_b(s):
        xs = jnp.concatenate([xs_ref[s * npair + q] for q in range(npair)], axis=0)
        bt = jax.lax.dot_general(pltpu.bitcast(wf_ref[1], bf16), pltpu.bitcast(xs, bf16), NT,
                                 preferred_element_type=f32)
        bt_ref[s] = pltpu.bitcast(bt.astype(bf16), u32)

    def qk_unit(t, p, q):
        def run():
            s = jnp.dot(pltpu.bitcast(at_ref[p], bf16), x_tile(0, t), preferred_element_type=f32)
            ref, r0, c0 = eloc(t)
            if isinstance(q, int):
                ref[0, r0 + q * PK:r0 + (q + 1) * PK, c0:c0 + LANE] = s
            else:
                ref[0, pl.ds(pl.multiple_of(r0 + q * PK, 8), PK), c0:c0 + LANE] = s
            mp_ref[t] = jnp.maximum(mp_ref[t], _colmax(s))
        return run

    def pv_units(s, zero):
        never = zero != 0
        st = {}

        def unit(t, j):
            def run():
                ref, r0, c0 = eloc(t)
                if j == 0:
                    m_old = m_ref[t]
                    m = jnp.maximum(_allmax(mp_ref[t]), m_old)
                    m_ref[t] = m
                    mp_ref[t] = m
                    st[t] = (m, jnp.exp2(m_old - m), zero, None)
                m, al, l, acc = st[t]
                l, acc = _pv_unit(ref[0, r0 + j * LANE:r0 + (j + 1) * LANE, c0:c0 + LANE], m, l, acc,
                                  bt_ref[s, :, j * LANE:(j + 1) * LANE], never)
                st[t] = (m, al, l, acc)
                if j == kts - 1:
                    alpha = jnp.where(never, acc[0:8, :], al)
                    acc_ref[t] = acc + (acc_ref[t].reshape(C // 8, 8, LANE) * alpha[None]).reshape(C, LANE)
                    l_ref[t] = l + l_ref[t] * alpha
            return run

        return [unit(t, j) for t in range(nte) for j in range(kts)]

    @pl.when(step == 0)
    def _early():
        wcp = [pltpu.make_async_copy(a, b, wsem.at[0])
               for a, b in ((wq_hbm, wq_ref), (wkv_hbm, wkv_ref), (wo_hbm, wo_ref))]
        for c_ in wcp:
            c_.start()
        xcopy(0).start()
        for c_ in wcp:
            c_.wait()
        for p in range(1, NS * npair):
            xcopy(p).start()
        zi_ref[0] = 0
        for s_ in sr:
            s_[0, NK:NK + 8, :] = jnp.zeros((8, TQ), f32)

        def init(i, c):
            ts = pl.ds(i * 4, 4)
            m_ref[ts] = jnp.full((4, 8, LANE), -jnp.inf, f32)
            mp_ref[ts] = jnp.full((4, 8, LANE), -jnp.inf, f32)
            l_ref[ts] = jnp.zeros((4, 8, LANE), f32)
            acc_ref[ts] = jnp.zeros((4, C, LANE), f32)
            return c
        jax.lax.fori_loop(0, nte // 4, init, 0)

        wa = jax.lax.dot_general(wkv_ref[:, :C], wq_ref[...], NT, preferred_element_type=f32)
        wa = wa * (C ** -0.5 * math.log2(math.e))
        wb = jnp.dot(wkv_ref[:, C:], wo_ref[...], preferred_element_type=f32)
        wf_ref[0] = pltpu.bitcast(wa.astype(bf16), u32)
        wf_ref[1] = pltpu.bitcast(wb.T.astype(bf16), u32)
        xcopy(0).wait()
        _interleave([], pool_events(0, 0, 0))

        def stage(s, carry):
            def quarter(q, c):
                p = s * npair + q
                xcopy(p + 1).wait()
                _interleave([qk_unit(t, p, q) for t in range(nte - late)], pool_events(p + 1, off, gap))
                return c
            jax.lax.fori_loop(0, npair - 1, quarter, 0)

            @pl.when(s + 1 < NS)
            def _():
                xcopy((s + 1) * npair).wait()
            nxt = jnp.minimum(s + 1, NS - 1) * npair
            q = npair - 1
            units = [(-2 if t < skew_e else (t - skew_e) * kts, 0, qk_unit(t, s * npair + q, q))
                     for t in range(nte)]
            units += [(-1, qq * nte + t, qk_unit(t, s * npair + qq, qq))
                      for qq in range(q) for t in range(nte - late, nte)]
            units += [(i, 1, u) for i, u in enumerate(pv_units(s, opaque_zero()))]
            units.sort(key=lambda e: e[:2])
            extra = pool_events(s * npair + npair, off2, gap2, prow=nxt)
            _interleave([u[2] for u in units], extra + [(pb_pos, 2, lambda: proj_b(s))])
            return carry
        jax.lax.fori_loop(0, NS, stage, 0)

    @pl.when(step >= 1)
    def _main():
        row0 = RE + (step - 1) * R
        ntile = R * wt
        nkt = NK // LANE
        zero = opaque_zero()
        never = zero != 0
        mx, xq, st = {}, {}, {}

        def at_rows(a, b):
            parts = []
            while a < b:
                p, o = divmod(a, PK)
                e = min(b - a, PK - o)
                parts.append(at_ref[p, o // 2:(o + e) // 2, :])
                a += e
            return parts[0] if len(parts) == 1 else jnp.concatenate(parts, axis=0)

        def qk(g, j):
            if g not in xq:
                xq[g] = jnp.concatenate([x_tile(row0, g * tpg + t) for t in range(tpg)], axis=1)
            s = jnp.dot(pltpu.bitcast(at_rows(j * LANE, (j + 1) * LANE), bf16), xq[g],
                        preferred_element_type=f32)
            sr[g % 3][0, j * LANE:(j + 1) * LANE, :] = s
            mj = _colmax(s)
            mx[g] = mj if j == 0 else jnp.maximum(mx[g], mj)
            if j == nkt - 1:
                mx[g] = _allmax(mx[g])

        def pv(t, j):
            g, u = divmod(t, tpg)
            us = slice(u * LANE, (u + 1) * LANE)
            l, acc = st.get(t, (zero, None))
            l, acc = _pv_unit(sr[g % 3][0, j * LANE:(j + 1) * LANE, us], mx[g][:, us], l, acc,
                              bt_ref[j // kts, :, (j % kts) * LANE:(j % kts + 1) * LANE], never)
            st[t] = (l, acc)
            if j == nkt - 1:
                normalise(row0, t, acc, l)
                if t + 1 == (R - RO) * wt:
                    ocopy(row0, R - RO).start()
                if t + 1 == ntile:
                    ocopy(row0 + R - RO, RO).start()

        def early_out(t, _):
            k = step - 1
            src = jnp.minimum(k, nev - 1) * (NR * wt) + t
            normalise(jnp.where(k < nev, k * NR, H), t, acc_ref[src], l_ref[src])

        events = [(i * tpg, 0, i, qk, divmod(i, nkt)) for i in range(ntile // tpg * nkt)]
        events += [(nkt * tpg + skew + (i // 4) * 4, 1, i, pv, divmod(i, nkt)) for i in range(ntile * nkt)]
        events += [((2 + 2 * t) * tpg, 2, t, early_out, (t, 0)) for t in range(NR * wt)]
        events.sort(key=lambda e: e[:3])
        for e in events:
            e[3](*e[4])

    @pl.when(step == nev)
    def _():
        ocopy(0, RE).start()

    @pl.when(step == pl.num_programs(0) - 1)
    def _():
        ocopy(0, H).wait()


@jax.jit
def pallas_standalone__window_attn_twins__vision_kernel(x, wq, wkv, wo):
    B, H, W, C = x.shape
    nk = (H // WIN) * (W // WIN)
    pk = 2 * W // WIN
    nte = RE * W // LANE
    nsteps = (H - RE) // R
    assert B == 1 and nk % SK == 0 and SK % pk == 0 and W % LANE == 0 and C % 16 == 0
    assert (H - RE) % R == 0 and RE <= 4 * WIN and nsteps >= RE // NR
    nb = max(3, -(-nte // ((nk // SK) * (TQ // LANE))))
    xt = jnp.transpose(x, (0, 1, 3, 2)).reshape(H, C, W)
    out = pl.pallas_call(
        functools.partial(_kernel, H=H, W=W, C=C, **CFG),
        grid=(1 + nsteps,),
        in_specs=[pl.BlockSpec(memory_space=pl.ANY)] * 4,
        out_specs=pl.BlockSpec(memory_space=pl.ANY),
        out_shape=jax.ShapeDtypeStruct((H, C, W), x.dtype),
        scratch_shapes=[
            pltpu.VMEM((H + NR, C, W), bf16), pltpu.SemaphoreType.DMA((1,)),
            pltpu.VMEM((H, C, W), bf16), pltpu.SemaphoreType.DMA((nk // pk,)),
            pltpu.VMEM((C, C), bf16), pltpu.VMEM((C, 2 * C), bf16), pltpu.VMEM((C, C), bf16),
            pltpu.SemaphoreType.DMA((1,)),
            pltpu.VMEM((nk // pk + 1, pk // 2, C), u32),
            pltpu.VMEM((nk // SK, C // 2, SK), u32),
            pltpu.VMEM((2, C // 2, C), u32),
            pltpu.VMEM((nk // pk, pk // 2, C), u32),
            pltpu.SMEM((1,), jnp.int32),
            pltpu.VMEM((nte, 8, LANE), f32), pltpu.VMEM((nte, 8, LANE), f32),
            pltpu.VMEM((nte, 8, LANE), f32), pltpu.VMEM((nte, C, LANE), f32),
        ] + [pltpu.VMEM((1, nk + 8, TQ), f32)] * nb,
        compiler_params=pltpu.CompilerParams(
            dimension_semantics=("arbitrary",),
            vmem_limit_bytes=110 * 1024 * 1024,
        ),
    )(xt, wq, wkv, wo)
    return jnp.transpose(out.reshape(1, H, C, W), (0, 1, 3, 2))
```

```python
import functools
import math

import jax
import jax.numpy as jnp
import jax.experimental.pallas as pl
import jax.experimental.pallas.tpu as pltpu

f32, bf16, u32 = jnp.float32, jnp.bfloat16, jnp.uint32
WIN = 8
LANE = 128
NT = (((1,), (1,)), ((), ()))

R = 16
RE = 32
SK = 384
TQ = 512
KP = 256
NR = 2
RO = 3
CFG = dict(skew=16, gap=3, off=2, dly1=2, dly=8, gap2=4, skew_e=6, off2=6, pb_pos=10, late=8)


def _colmax(s):
    return jnp.max(s.reshape(s.shape[0] // 8, 8, s.shape[1]), axis=0)


def _allmax(m):
    return jnp.broadcast_to(jnp.max(m, axis=0, keepdims=True), m.shape)


def _pv_block(sv, m, l, acc, bt, never):
    nk = sv.shape[0]
    p = jnp.exp2(sv.reshape(nk // LANE, LANE // 8, 8, LANE) - m[None, None])
    ps = jnp.sum(p, axis=1)
    parts = []
    for k in range(nk // LANE):
        l = l + ps[k]
        parts += [jnp.where(never, l, p[k, 0])[None], p[k, 1:]]
    p = jnp.concatenate(parts, axis=0).reshape(nk, LANE)
    o = jnp.dot(pltpu.bitcast(bt, bf16), p.astype(bf16), preferred_element_type=f32)
    return l, (o if acc is None else o + acc)


def _interleave(main, extra):
    extra = sorted(extra, key=lambda e: e[:2])
    for i, fn in enumerate(main):
        while extra and extra[0][0] <= i:
            extra.pop(0)[2]()
        fn()
    for e in extra:
        e[2]()


def _kernel(x_hbm, wq_hbm, wkv_hbm, wo_hbm, o_hbm,
            o_vm, osem, x_vm, xsems, wq_ref, wkv_ref, wo_ref, wsem, at_ref, bt_ref, wf_ref, xs_ref,
            zi_ref, mp_ref, m_ref, l_ref, acc_ref, *sr,
            H, W, C, skew, gap, off, dly, gap2, skew_e, off2, pb_pos, late, dly1):
    step = pl.program_id(0)
    NS = bt_ref.shape[0]
    NK = NS * SK
    PK = 2 * W // WIN
    rpp = 2 * WIN
    npair = SK // PK
    wt = W // LANE
    tpg = TQ // LANE
    NB = len(sr)
    nte = RE * wt
    nev = RE // NR

    def xcopy(p):
        rows = pl.ds(p * rpp, rpp)
        return pltpu.make_async_copy(x_hbm.at[rows], x_vm.at[rows], xsems.at[p])

    def ocopy(r0, n):
        rows = pl.ds(r0, n)
        return pltpu.make_async_copy(o_vm.at[rows], o_hbm.at[rows], osem.at[0])

    def opaque_zero():
        zd = zi_ref[0]
        return sum(s_[zd, NK:NK + 8, 0:LANE] for s_ in sr)

    def x_tile(row0, t):
        return x_vm[row0 + t // wt, :, (t % wt) * LANE:(t % wt + 1) * LANE]

    def normalise(row0, t, acc, l):
        r, c = divmod(t, wt)
        lt = jnp.sum(l, axis=0, keepdims=True)
        o_vm[row0 + r, :, c * LANE:(c + 1) * LANE] = (acc * (1.0 / lt)).astype(o_vm.dtype)

    def eloc(t):
        g, u = divmod(t, tpg)
        return sr[g % NB], (g // NB) * SK, u * LANE

    def pool_events(p, pos0, gap_, dly_, prow=None):
        kpt = LANE // WIN
        jj = jax.lax.broadcasted_iota(jnp.int32, (kpt, LANE), 0)
        ww = jax.lax.broadcasted_iota(jnp.int32, (kpt, LANE), 1)
        pool = jnp.where((ww >= jj * WIN) & (ww < (jj + 1) * WIN), 1.0 / (WIN * WIN), 0.0).astype(bf16)
        prow = p if prow is None else prow
        means = {}

        def piece(k):
            def run():
                i, c = divmod(k, wt)
                blk = x_vm[pl.ds(prow * rpp + i * WIN, WIN), :, c * LANE:(c + 1) * LANE]
                ssum = jnp.sum(blk.astype(f32), axis=0)
                hi = ssum.astype(bf16)
                lo = (ssum - hi.astype(f32)).astype(bf16)
                r = jax.lax.dot_general(pool, hi, NT, preferred_element_type=f32)
                r = jax.lax.dot_general(pool, lo, NT, preferred_element_type=f32) + r
                means[k] = r.astype(bf16)
            return run

        def proj():
            xs = jnp.concatenate([means[k] for k in range(2 * wt)], axis=0)
            xs_ref[prow] = pltpu.bitcast(xs, u32)
            at = jnp.dot(xs, pltpu.bitcast(wf_ref[0], bf16), preferred_element_type=f32)
            at_ref[p] = pltpu.bitcast(at.astype(bf16), u32)

        ev = [(pos0 + k * gap_, 0, piece(k)) for k in range(2 * wt)]
        ev.append((pos0 + (2 * wt - 1) * gap_ + dly_, 1, proj))
        return ev

    def proj_b(s):
        xs = jnp.concatenate([xs_ref[s * npair + q] for q in range(npair)], axis=0)
        bt = jax.lax.dot_general(pltpu.bitcast(wf_ref[1], bf16), pltpu.bitcast(xs, bf16), NT,
                                 preferred_element_type=f32)
        bt_ref[s] = pltpu.bitcast(bt.astype(bf16), u32)

    def qk_unit(t, p, q, n=1):
        def run():
            xt = jnp.concatenate([x_tile(0, t + i) for i in range(n)], axis=1)
            s = jnp.dot(pltpu.bitcast(at_ref[p], bf16), xt, preferred_element_type=f32)
            ref, r0, c0 = eloc(t)
            cols = slice(c0, c0 + n * LANE)
            if isinstance(q, int):
                ref[0, r0 + q * PK:r0 + (q + 1) * PK, cols] = s
            else:
                ref[0, pl.ds(pl.multiple_of(r0 + q * PK, 8), PK), cols] = s
            mp_ref[t // tpg, :, cols] = jnp.maximum(mp_ref[t // tpg, :, cols], _colmax(s))
        return run

    def pv_tile(t, s, zero):
        def run():
            never = zero != 0
            ref, r0, c0 = eloc(t)
            m_old = m_ref[t]
            m = _allmax(mp_ref[t // tpg, :, c0:c0 + LANE])
            m_ref[t] = m
            alpha = jnp.exp2(m_old - m)
            l, acc = _pv_block(ref[0, r0:r0 + SK, c0:c0 + LANE], m, zero, None, bt_ref[s], never)
            alpha = jnp.where(never, acc[0:8, :], alpha)
            acc_ref[t] = acc + (acc_ref[t].reshape(C // 8, 8, LANE) * alpha[None]).reshape(C, LANE)
            l_ref[t] = l + l_ref[t] * alpha
        return run

    @pl.when(step == 0)
    def _early():
        wcp = [pltpu.make_async_copy(a, b, wsem.at[0])
               for a, b in ((wq_hbm, wq_ref), (wkv_hbm, wkv_ref), (wo_hbm, wo_ref))]
        for c_ in wcp:
            c_.start()
        xcopy(0).start()
        for c_ in wcp:
            c_.wait()
        for p in range(1, NS * npair):
            xcopy(p).start()
        zi_ref[0] = 0
        for s_ in sr:
            s_[0, NK:NK + 8, :] = jnp.zeros((8, TQ), f32)

        def init(i, c):
            ts = pl.ds(i * tpg, tpg)
            m_ref[ts] = jnp.full((tpg, 8, LANE), -jnp.inf, f32)
            mp_ref[i] = jnp.full((8, TQ), -jnp.inf, f32)
            l_ref[ts] = jnp.zeros((tpg, 8, LANE), f32)
            acc_ref[ts] = jnp.zeros((tpg, C, LANE), f32)
            return c
        jax.lax.fori_loop(0, nte // tpg, init, 0)

        wa = jax.lax.dot_general(wkv_ref[:, :C], wq_ref[...], NT, preferred_element_type=f32)
        wa = wa * (C ** -0.5 * math.log2(math.e))
        wb = jnp.dot(wkv_ref[:, C:], wo_ref[...], preferred_element_type=f32)
        wf_ref[0] = pltpu.bitcast(wa.astype(bf16), u32)
        wf_ref[1] = pltpu.bitcast(wb.T.astype(bf16), u32)
        xcopy(0).wait()
        _interleave([], pool_events(0, 0, 0, 0))

        def stage(s, carry):
            def quarter(q, c):
                p = s * npair + q
                xcopy(p + 1).wait()
                _interleave([qk_unit(t, p, q, tpg) for t in range(0, nte - late, tpg)],
                            pool_events(p + 1, off, gap, dly1))
                return c
            jax.lax.fori_loop(0, npair - 1, quarter, 0)

            @pl.when(s + 1 < NS)
            def _():
                xcopy((s + 1) * npair).wait()
            nxt = jnp.minimum(s + 1, NS - 1) * npair
            q = npair - 1
            units = [(-2 if t < skew_e else t - skew_e, 0, qk_unit(t, s * npair + q, q))
                     for t in range(nte)]
            units += [(-1, qq * nte + t, qk_unit(t, s * npair + qq, qq))
                      for qq in range(q) for t in range(nte - late, nte)]
            zero = opaque_zero()
            units += [(t, 1, pv_tile(t, s, zero)) for t in range(nte)]
            units.sort(key=lambda e: e[:2])
            extra = pool_events(s * npair + npair, off2, gap2, dly, prow=nxt)
            _interleave([u[2] for u in units], extra + [(pb_pos, 2, lambda: proj_b(s))])
            return carry
        jax.lax.fori_loop(0, NS, stage, 0)

    @pl.when(step >= 1)
    def _main():
        row0 = RE + (step - 1) * R
        ntile = R * wt
        nkt = NK // LANE
        zero = opaque_zero()
        never = zero != 0
        mx, xq, st = {}, {}, {}

        def at_rows(a, b):
            parts = []
            while a < b:
                p, o = divmod(a, PK)
                e = min(b - a, PK - o)
                parts.append(at_ref[p, o // 2:(o + e) // 2, :])
                a += e
            return parts[0] if len(parts) == 1 else jnp.concatenate(parts, axis=0)

        def qk(g, j):
            if g not in xq:
                xq[g] = jnp.concatenate([x_tile(row0, g * tpg + t) for t in range(tpg)], axis=1)
            s = jnp.dot(pltpu.bitcast(at_rows(j * LANE, (j + 1) * LANE), bf16), xq[g],
                        preferred_element_type=f32)
            sr[g % 3][0, j * LANE:(j + 1) * LANE, :] = s
            mj = _colmax(s)
            mx[g] = mj if j == 0 else jnp.maximum(mx[g], mj)
            if j == nkt - 1:
                mx[g] = _allmax(mx[g])

        def bt_cols(a, b):
            parts = []
            while a < b:
                s_, o = divmod(a, SK)
                e = min(b - a, SK - o)
                parts.append(bt_ref[s_, :, o:o + e])
                a += e
            return parts[0] if len(parts) == 1 else jnp.concatenate(parts, axis=1)

        def pv(t, j):
            g, u = divmod(t, tpg)
            us = slice(u * LANE, (u + 1) * LANE)
            l, acc = st.get(t, (zero, None))
            l, acc = _pv_block(sr[g % 3][0, j * KP:(j + 1) * KP, us], mx[g][:, us], l, acc,
                               bt_cols(j * KP, (j + 1) * KP), never)
            st[t] = (l, acc)
            if j == NK // KP - 1:
                normalise(row0, t, acc, l)
                if t + 1 == (R - RO) * wt:
                    ocopy(row0, R - RO).start()
                if t + 1 == ntile:
                    ocopy(row0 + R - RO, RO).start()

        def early_out(t, _):
            k = step - 1
            src = jnp.minimum(k, nev - 1) * (NR * wt) + t
            normalise(jnp.where(k < nev, k * NR, H), t, acc_ref[src], l_ref[src])

        events = [(i * tpg, 0, i, qk, divmod(i, nkt)) for i in range(ntile // tpg * nkt)]
        events += [(nkt * tpg + skew + (i * KP // TQ) * tpg, 1, i, pv, divmod(i, NK // KP))
                   for i in range(ntile * NK // KP)]
        events += [((2 + 2 * t) * tpg, 2, t, early_out, (t, 0)) for t in range(NR * wt)]
        events.sort(key=lambda e: e[:3])
        for e in events:
            e[3](*e[4])

    @pl.when(step == nev)
    def _():
        ocopy(0, RE).start()

    @pl.when(step == pl.num_programs(0) - 1)
    def _():
        ocopy(0, H).wait()


@jax.jit
def pallas_standalone__window_attn_twins__vision_kernel(x, wq, wkv, wo):
    B, H, W, C = x.shape
    nk = (H // WIN) * (W // WIN)
    pk = 2 * W // WIN
    nte = RE * W // LANE
    nsteps = (H - RE) // R
    assert B == 1 and nk % SK == 0 and SK % pk == 0 and W % LANE == 0 and C % 16 == 0
    assert (H - RE) % R == 0 and RE <= 4 * WIN and nsteps >= RE // NR
    nb = max(3, -(-nte // ((nk // SK) * (TQ // LANE))))
    xt = jnp.transpose(x, (0, 1, 3, 2)).reshape(H, C, W)
    out = pl.pallas_call(
        functools.partial(_kernel, H=H, W=W, C=C, **CFG),
        grid=(1 + nsteps,),
        in_specs=[pl.BlockSpec(memory_space=pl.ANY)] * 4,
        out_specs=pl.BlockSpec(memory_space=pl.ANY),
        out_shape=jax.ShapeDtypeStruct((H, C, W), x.dtype),
        scratch_shapes=[
            pltpu.VMEM((H + NR, C, W), bf16), pltpu.SemaphoreType.DMA((1,)),
            pltpu.VMEM((H, C, W), bf16), pltpu.SemaphoreType.DMA((nk // pk,)),
            pltpu.VMEM((C, C), bf16), pltpu.VMEM((C, 2 * C), bf16), pltpu.VMEM((C, C), bf16),
            pltpu.SemaphoreType.DMA((1,)),
            pltpu.VMEM((nk // pk + 1, pk // 2, C), u32),
            pltpu.VMEM((nk // SK, C // 2, SK), u32),
            pltpu.VMEM((2, C // 2, C), u32),
            pltpu.VMEM((nk // pk, pk // 2, C), u32),
            pltpu.SMEM((1,), jnp.int32),
            pltpu.VMEM((nte * LANE // TQ, 8, TQ), f32), pltpu.VMEM((nte, 8, LANE), f32),
            pltpu.VMEM((nte, 8, LANE), f32), pltpu.VMEM((nte, C, LANE), f32),
        ] + [pltpu.VMEM((1, nk + 8, TQ), f32)] * nb,
        compiler_params=pltpu.CompilerParams(
            dimension_semantics=("arbitrary",),
            vmem_limit_bytes=110 * 1024 * 1024,
        ),
    )(xt, wq, wkv, wo)
    return jnp.transpose(out.reshape(1, H, C, W), (0, 1, 3, 2))
```

```python
import functools
import math

import jax
import jax.numpy as jnp
import jax.experimental.pallas as pl
import jax.experimental.pallas.tpu as pltpu

f32, bf16, u32 = jnp.float32, jnp.bfloat16, jnp.uint32
WIN = 8
LANE = 128
NT = (((1,), (1,)), ((), ()))

R = 16
RE = 32
SK = 384
TQ = 512
KP = 256
NR = 2
RO = 3
NV = 48
NG = 3
CFG = dict(t0=280, t1=100, tl=400, t00=150, gap=3, off=2, dly1=2, dly=8, gap2=4, skew_e=6, off2=6, pb_pos=10, late=8)


def _colmax(s):
    return jnp.max(s.reshape(s.shape[0] // 8, 8, s.shape[1]), axis=0)


def _allmax(m):
    return jnp.broadcast_to(jnp.max(m, axis=0, keepdims=True), m.shape)


def _pv_block(sv, m, l, acc, bt, never):
    nk = sv.shape[0]
    p = jnp.exp2(sv.reshape(nk // LANE, LANE // 8, 8, LANE) - m[None, None])
    ps = jnp.sum(p, axis=1)
    parts = []
    for k in range(nk // LANE):
        l = l + ps[k]
        parts += [jnp.where(never, l, p[k, 0])[None], p[k, 1:]]
    p = jnp.concatenate(parts, axis=0).reshape(nk, LANE)
    o = jnp.dot(pltpu.bitcast(bt, bf16), p.astype(bf16), preferred_element_type=f32)
    return l, (o if acc is None else o + acc)


def _vpu_scores(xf, ab_ref, row0, never):
    sub = jax.lax.broadcasted_iota(jnp.int32, (NG, 8, LANE), 1)
    xv = xf.reshape(1, xf.shape[0] // 8, 8, LANE)

    def merge(a, b, s):
        low = (sub & s) == 0
        if s == 4:
            return jnp.where(low, a, b) + pltpu.roll(jnp.where(low, b, a), 4, 1)
        return jnp.where(low, a + pltpu.roll(a, 8 - s, 1), b + pltpu.roll(b, s, 1))

    stack, acc = [], None
    for n in range(8):
        p = ab_ref[row0 + n] * xv
        if acc is not None:
            p = jnp.concatenate([jnp.where(never, acc, p[:, 0])[:, None], p[:, 1:]], axis=1)
        acc = jnp.sum(p, axis=1)
        lvl = 0
        while stack and stack[-1][0] == lvl:
            acc = merge(stack.pop()[1], acc, 4 >> lvl)
            lvl += 1
        stack.append((lvl, acc))
    return acc


def _interleave(main, extra):
    extra = sorted(extra, key=lambda e: e[:2])
    for i, fn in enumerate(main):
        while extra and extra[0][0] <= i:
            extra.pop(0)[2]()
        fn()
    for e in extra:
        e[2]()


def _kernel(x_hbm, wq_hbm, wkv_hbm, wo_hbm, o_hbm,
            oe_vm, osem, x_vm, xsems, wq_ref, wkv_ref, wo_ref, wsem, at_ref, bt_ref, wf_ref, xs_ref,
            zi_ref, mp_ref, m_ref, l_ref, acc_ref, ab_ref, *sr,
            H, W, C, t0, t1, tl, t00, gap, off, dly, gap2, skew_e, off2, pb_pos, late, dly1):
    step = pl.program_id(0)
    NS = bt_ref.shape[0]
    NK = NS * SK
    PK = 2 * W // WIN
    rpp = 2 * WIN
    npair = SK // PK
    wt = W // LANE
    tpg = TQ // LANE
    nte = RE * wt
    nev = RE // NR
    NBE = -(-nte // (NS * tpg))

    def xcopy(p):
        rows = pl.ds(p * rpp, rpp)
        return pltpu.make_async_copy(x_hbm.at[rows], x_vm.at[rows], xsems.at[p])

    def ocopy(buf, r0, n):
        rows = pl.ds(r0, n)
        return pltpu.make_async_copy(buf.at[rows], o_hbm.at[rows], osem.at[0])

    def opaque_zero(n):
        zd = zi_ref[0]
        return sum(s_[zd, NK:NK + 8, 0:LANE] for s_ in sr[:n])

    def x_tile(row0, t):
        return x_vm[row0 + t // wt, :, (t % wt) * LANE:(t % wt + 1) * LANE]

    def normalise(buf, row0, t, acc, l):
        r, c = divmod(t, wt)
        lt = jnp.sum(l, axis=0, keepdims=True)
        buf[row0 + r, :, c * LANE:(c + 1) * LANE] = (acc * (1.0 / lt)).astype(buf.dtype)

    def eloc(t):
        g, u = divmod(t, tpg)
        return sr[g % NBE], (g // NBE) * SK, u * LANE

    def pool_events(p, pos0, gap_, dly_, prow=None):
        kpt = LANE // WIN
        jj = jax.lax.broadcasted_iota(jnp.int32, (kpt, LANE), 0)
        ww = jax.lax.broadcasted_iota(jnp.int32, (kpt, LANE), 1)
        pool = jnp.where((ww >= jj * WIN) & (ww < (jj + 1) * WIN), 1.0 / (WIN * WIN), 0.0).astype(bf16)
        prow = p if prow is None else prow
        means = {}

        def piece(k):
            def run():
                i, c = divmod(k, wt)
                blk = x_vm[pl.ds(prow * rpp + i * WIN, WIN), :, c * LANE:(c + 1) * LANE]
                ssum = jnp.sum(blk.astype(f32), axis=0)
                hi = ssum.astype(bf16)
                lo = (ssum - hi.astype(f32)).astype(bf16)
                r = jax.lax.dot_general(pool, hi, NT, preferred_element_type=f32)
                r = jax.lax.dot_general(pool, lo, NT, preferred_element_type=f32) + r
                means[k] = r.astype(bf16)
            return run

        def proj():
            xs = jnp.concatenate([means[k] for k in range(2 * wt)], axis=0)
            xs_ref[prow] = pltpu.bitcast(xs, u32)
            at = jnp.dot(xs, pltpu.bitcast(wf_ref[0], bf16), preferred_element_type=f32)
            at_ref[p] = pltpu.bitcast(at.astype(bf16), u32)

        ev = [(pos0 + k * gap_, 0, piece(k)) for k in range(2 * wt)]
        ev.append((pos0 + (2 * wt - 1) * gap_ + dly_, 1, proj))
        return ev

    def proj_b(s):
        xs = jnp.concatenate([xs_ref[s * npair + q] for q in range(npair)], axis=0)
        bt = jax.lax.dot_general(pltpu.bitcast(wf_ref[1], bf16), pltpu.bitcast(xs, bf16), NT,
                                 preferred_element_type=f32)
        bt_ref[s] = pltpu.bitcast(bt.astype(bf16), u32)

    def qk_unit(t, p, q, n=1):
        def run():
            xt = jnp.concatenate([x_tile(0, t + i) for i in range(n)], axis=1)
            s = jnp.dot(pltpu.bitcast(at_ref[p], bf16), xt, preferred_element_type=f32)
            ref, r0, c0 = eloc(t)
            cols = slice(c0, c0 + n * LANE)
            if isinstance(q, int):
                ref[0, r0 + q * PK:r0 + (q + 1) * PK, cols] = s
            else:
                ref[0, pl.ds(pl.multiple_of(r0 + q * PK, 8), PK), cols] = s
            mp_ref[t // tpg, :, cols] = jnp.maximum(mp_ref[t // tpg, :, cols], _colmax(s))
        return run

    def pv_tile(t, s, zero):
        def run():
            never = zero != 0
            ref, r0, c0 = eloc(t)
            m_old = m_ref[t]
            m = _allmax(mp_ref[t // tpg, :, c0:c0 + LANE])
            m_ref[t] = m
            alpha = jnp.exp2(m_old - m)
            l, acc = _pv_block(ref[0, r0:r0 + SK, c0:c0 + LANE], m, zero, None, bt_ref[s], never)
            alpha = jnp.where(never, acc[0:8, :], alpha)
            acc_ref[t] = acc + (acc_ref[t].reshape(C // 8, 8, LANE) * alpha[None]).reshape(C, LANE)
            l_ref[t] = l + l_ref[t] * alpha
        return run

    @pl.when(step == 0)
    def _early():
        wcp = [pltpu.make_async_copy(a, b, wsem.at[0])
               for a, b in ((wq_hbm, wq_ref), (wkv_hbm, wkv_ref), (wo_hbm, wo_ref))]
        for c_ in wcp:
            c_.start()
        xcopy(0).start()
        for c_ in wcp:
            c_.wait()
        for p in range(1, NS * npair):
            xcopy(p).start()
        zi_ref[0] = 0
        for s_ in sr:
            s_[0, NK:NK + 8, :] = jnp.zeros((8, TQ), f32)

        def init(i, c):
            ts = pl.ds(i * tpg, tpg)
            m_ref[ts] = jnp.full((tpg, 8, LANE), -jnp.inf, f32)
            mp_ref[i] = jnp.full((8, TQ), -jnp.inf, f32)
            l_ref[ts] = jnp.zeros((tpg, 8, LANE), f32)
            acc_ref[ts] = jnp.zeros((tpg, C, LANE), f32)
            return c
        jax.lax.fori_loop(0, nte // tpg, init, 0)

        wa = jax.lax.dot_general(wkv_ref[:, :C], wq_ref[...], NT, preferred_element_type=f32)
        wa = wa * (C ** -0.5 * math.log2(math.e))
        wb = jnp.dot(wkv_ref[:, C:], wo_ref[...], preferred_element_type=f32)
        wf_ref[0] = pltpu.bitcast(wa.astype(bf16), u32)
        wf_ref[1] = pltpu.bitcast(wb.T.astype(bf16), u32)
        wf_ref[2] = pltpu.bitcast(wa.T.astype(bf16), u32)
        xcopy(0).wait()
        _interleave([], pool_events(0, 0, 0, 0))
        att = jax.lax.dot_general(pltpu.bitcast(wf_ref[2], bf16), pltpu.bitcast(xs_ref[0], bf16), NT,
                                  preferred_element_type=f32)
        for k in range(NV):
            blk, r = divmod(k, 8 * NG)
            n = int(format(r % 8, "03b")[::-1], 2)
            col = jnp.broadcast_to(att[:, k:k + 1], (C, LANE))
            ab_ref[blk * 8 + n, r // 8] = col.reshape(C // 8, 8, LANE)

        def stage(s, carry):
            def quarter(q, c):
                p = s * npair + q
                xcopy(p + 1).wait()
                _interleave([qk_unit(t, p, q, tpg) for t in range(0, nte - late, tpg)],
                            pool_events(p + 1, off, gap, dly1))
                return c
            jax.lax.fori_loop(0, npair - 1, quarter, 0)

            @pl.when(s + 1 < NS)
            def _():
                xcopy((s + 1) * npair).wait()
            nxt = jnp.minimum(s + 1, NS - 1) * npair
            q = npair - 1
            units = [(-2 if t < skew_e else t - skew_e, 0, qk_unit(t, s * npair + q, q))
                     for t in range(nte)]
            units += [(-1, qq * nte + t, qk_unit(t, s * npair + qq, qq))
                      for qq in range(q) for t in range(nte - late, nte)]
            zero = opaque_zero(NBE)
            units += [(t, 1, pv_tile(t, s, zero)) for t in range(nte)]
            units.sort(key=lambda e: e[:2])
            extra = pool_events(s * npair + npair, off2, gap2, dly, prow=nxt)
            _interleave([u[2] for u in units], extra + [(pb_pos, 2, lambda: proj_b(s))])
            return carry
        jax.lax.fori_loop(0, NS, stage, 0)

    @pl.when(step >= 1)
    def _main():
        row0 = RE + (step - 1) * R
        ntile = R * wt
        G = ntile // tpg
        NM = NK - NV
        npc = tpg * NV // (8 * NG)
        zero = opaque_zero(G)
        never = zero != 0
        mx, vm = {}, {}
        last = step == pl.num_programs(0) - 1

        def at_rows(a, b):
            parts = []
            while a < b:
                p, o = divmod(a, PK)
                e = min(b - a, PK - o)
                parts.append(at_ref[p, o // 2:(o + e) // 2, :])
                a += e
            return parts[0] if len(parts) == 1 else jnp.concatenate(parts, axis=0)

        def bt_cols(a, b):
            parts = []
            while a < b:
                s_, o = divmod(a, SK)
                e = min(b - a, SK - o)
                parts.append(bt_ref[s_, :, o:o + e])
                a += e
            return parts[0] if len(parts) == 1 else jnp.concatenate(parts, axis=1)

        def early_out(t):
            k = step - 1
            src = jnp.minimum(k, nev - 1) * (NR * wt) + t
            normalise(oe_vm, jnp.minimum(k, nev) * NR, t, acc_ref[src], l_ref[src])

        for g in range(G):
            xq = jnp.concatenate([x_tile(row0, g * tpg + t) for t in range(tpg)], axis=1)
            lo, hi = (t00 if g == 0 else t0), NM - (t1 if g < G - 1 else tl)
            due = [int(lo + (hi - lo) * i / (npc - 1)) for i in range(npc)]
            for j in range(-(-NM // LANE)):
                a, b = NV + j * LANE, min(NV + (j + 1) * LANE, NK)
                s = jnp.dot(pltpu.bitcast(at_rows(a, b), bf16), xq, preferred_element_type=f32)
                for k in [k for k in range(npc) if due[k] // LANE == j]:
                    u, kb = divmod(k, npc // tpg)
                    sv = _vpu_scores(xq[:, u * LANE:(u + 1) * LANE].astype(f32), ab_ref, kb * 8, never)
                    r0 = kb * 8 * NG
                    sr[g][0, r0:r0 + 8 * NG, u * LANE:(u + 1) * LANE] = sv.reshape(8 * NG, LANE)
                    m = jnp.max(sv, axis=0)
                    vm.setdefault(g * tpg + u, []).append(m)
                    i = (due[k] % LANE) // 16 * 16
                    tied = jnp.concatenate([jnp.where(never, m, s[i:i + 8, :LANE]), s[i:i + 8, LANE:]], axis=1)
                    s = jnp.concatenate([v for v in (s[:i], tied, s[i + 8:]) if v.shape[0]], axis=0)
                sr[g][0, a:b, :] = s
                mx[g] = _colmax(s) if j == 0 else jnp.maximum(mx[g], _colmax(s))
                if j == 0 and 1 <= g <= NR * wt:
                    early_out(g - 1)

        for t in range(ntile):
            g, u = divmod(t, tpg)
            us = slice(u * LANE, (u + 1) * LANE)
            m = _allmax(functools.reduce(jnp.maximum, vm[t], mx[g][:, us]))
            l, acc = zero, None
            for j in range(NK // KP):
                l, acc = _pv_block(sr[g][0, j * KP:(j + 1) * KP, us], m, l, acc,
                                   bt_cols(j * KP, (j + 1) * KP), never)
            normalise(x_vm, row0, t, acc, l)
            if t + 1 == (R - RO) * wt:
                pl.when(last)(lambda: ocopy(x_vm, row0, R - RO).start())
        pl.when(last)(lambda: ocopy(x_vm, row0 + R - RO, RO).start())
        pl.when(jnp.logical_not(last))(lambda: ocopy(x_vm, row0, R).start())

    @pl.when(step == nev)
    def _():
        ocopy(oe_vm, 0, RE).start()

    @pl.when(step == pl.num_programs(0) - 1)
    def _():
        ocopy(x_vm, 0, H).wait()


@jax.jit
def pallas_standalone__window_attn_twins__vision_kernel(x, wq, wkv, wo):
    B, H, W, C = x.shape
    nk = (H // WIN) * (W // WIN)
    pk = 2 * W // WIN
    nte = RE * W // LANE
    nsteps = (H - RE) // R
    assert B == 1 and nk % SK == 0 and SK % pk == 0 and W % LANE == 0 and C % 16 == 0
    assert (H - RE) % R == 0 and RE <= 4 * WIN and nsteps >= RE // NR
    xt = jnp.transpose(x, (0, 1, 3, 2)).reshape(H, C, W)
    out = pl.pallas_call(
        functools.partial(_kernel, H=H, W=W, C=C, **CFG),
        grid=(1 + nsteps,),
        in_specs=[pl.BlockSpec(memory_space=pl.ANY)] * 4,
        out_specs=pl.BlockSpec(memory_space=pl.ANY),
        out_shape=jax.ShapeDtypeStruct((H, C, W), x.dtype),
        scratch_shapes=[
            pltpu.VMEM((RE + NR, C, W), bf16), pltpu.SemaphoreType.DMA((1,)),
            pltpu.VMEM((H, C, W), bf16), pltpu.SemaphoreType.DMA((nk // pk,)),
            pltpu.VMEM((C, C), bf16), pltpu.VMEM((C, 2 * C), bf16), pltpu.VMEM((C, C), bf16),
            pltpu.SemaphoreType.DMA((1,)),
            pltpu.VMEM((nk // pk + 1, pk // 2, C), u32),
            pltpu.VMEM((nk // SK, C // 2, SK), u32),
            pltpu.VMEM((3, C // 2, C), u32),
            pltpu.VMEM((nk // pk, pk // 2, C), u32),
            pltpu.SMEM((1,), jnp.int32),
            pltpu.VMEM((nte * LANE // TQ, 8, TQ), f32), pltpu.VMEM((nte, 8, LANE), f32),
            pltpu.VMEM((nte, 8, LANE), f32), pltpu.VMEM((nte, C, LANE), f32),
            pltpu.VMEM((NV // NG, NG, C // 8, 8, LANE), f32),
        ] + [pltpu.VMEM((1, nk + 8, TQ), f32)] * (R * W // TQ),
        compiler_params=pltpu.CompilerParams(
            dimension_semantics=("arbitrary",),
            vmem_limit_bytes=110 * 1024 * 1024,
        ),
    )(xt, wq, wkv, wo)
    return jnp.transpose(out.reshape(1, H, C, W), (0, 1, 3, 2))
```

```python
import functools
import itertools
import math

import jax
import jax.numpy as jnp
import jax.experimental.pallas as pl
import jax.experimental.pallas.tpu as pltpu

f32, bf16, u32 = jnp.float32, jnp.bfloat16, jnp.uint32
WIN = 8
LANE = 128
NT = (((1,), (1,)), ((), ()))

R = 16
RE = 32
SK = 384
TQ = 512
KP = 256
NR = 2
RO = 3
NVMAX = 64
CFG = dict(nsmall=2, t0=64, t1=8, tl=400, w1=250, f1=0.7,
           gap=3, off=2, dly1=2, dly=8, gap2=4, skew_e=6, off2=6, pb_pos=10, late=8)


def _colmax(s):
    return jnp.max(s.reshape(s.shape[0] // 8, 8, s.shape[1]), axis=0)


def _allmax(m):
    return jnp.broadcast_to(jnp.max(m, axis=0, keepdims=True), m.shape)


def _pv_block(sv, m, l, acc, bt, never):
    nk = sv.shape[0]
    p = jnp.exp2(sv.reshape(nk // LANE, LANE // 8, 8, LANE) - m[None, None])
    ps = jnp.sum(p, axis=1)
    parts = []
    for k in range(nk // LANE):
        l = l + ps[k]
        parts += [jnp.where(never, l, p[k, 0])[None], p[k, 1:]]
    p = jnp.concatenate(parts, axis=0).reshape(nk, LANE)
    o = jnp.dot(pltpu.bitcast(bt, bf16), p.astype(bf16), preferred_element_type=f32)
    return l, (o if acc is None else o + acc)


def _merge(a, b, s):
    ax = a.ndim - 2
    low = (jax.lax.broadcasted_iota(jnp.int32, a.shape, ax) & s) == 0
    if s == 4:
        return jnp.where(low, a, b) + pltpu.roll(jnp.where(low, b, a), 4, ax)
    return jnp.where(low, a + pltpu.roll(a, 8 - s, ax), b + pltpu.roll(b, s, ax))


def _vpu_scores(xt, ab):
    n = ab.shape[0] // 8
    xf = xt.astype(f32).reshape(1, xt.shape[0] // 8, 8, LANE)
    h = jnp.sum(ab * xf, axis=1).reshape(n * 4, 2, 8, LANE)
    p = _merge(h[:, 0], h[:, 1], 4).reshape(n * 2, 2, 8, LANE)
    q = _merge(p[:, 0], p[:, 1], 2).reshape(n, 2, 8, LANE)
    f = _merge(q[:, 0], q[:, 1], 1)
    pe = p[:, 0].reshape(n, 2, 8, LANE)
    return f, jnp.stack([pe[:, 0], q[:, 0], pe[:, 1], f], axis=1).reshape(n * 4, 8, LANE)


def _interleave(main, extra):
    extra = sorted(extra, key=lambda e: e[:2])
    for i, fn in enumerate(main):
        while extra and extra[0][0] <= i:
            extra.pop(0)[2]()
        fn()
    for e in extra:
        e[2]()


def _kernel(x_hbm, wq_hbm, wkv_hbm, wo_hbm, o_hbm,
            oe_vm, osem, x_vm, xsems, wq_ref, wkv_ref, wo_ref, wsem, at_ref, bt_ref, wf_ref, xs_ref,
            zi_ref, mp_ref, m_ref, l_ref, acc_ref, att_ref, ab_ref, *sr,
            H, W, C, nsmall, t0, t1, tl, w1, f1, gap, off, dly, gap2, skew_e, off2, pb_pos, late, dly1):
    step = pl.program_id(0)
    NS = bt_ref.shape[0]
    NK = NS * SK
    PK = 2 * W // WIN
    rpp = 2 * WIN
    npair = SK // PK
    wt = W // LANE
    tpg = TQ // LANE
    nte = RE * wt
    nev = RE // NR
    NBE = -(-nte // (NS * tpg))

    def xcopy(p):
        rows = pl.ds(p * rpp, rpp)
        return pltpu.make_async_copy(x_hbm.at[rows], x_vm.at[rows], xsems.at[p])

    def ocopy(buf, r0, n):
        rows = pl.ds(r0, n)
        return pltpu.make_async_copy(buf.at[rows], o_hbm.at[rows], osem.at[0])

    def opaque_zero(n):
        zd = zi_ref[0]
        return sum(s_[zd, NK:NK + 8, 0:LANE] for s_ in sr[:n])

    def x_tile(row0, t):
        return x_vm[row0 + t // wt, :, (t % wt) * LANE:(t % wt + 1) * LANE]

    def normalise(buf, row0, t, acc, l):
        r, c = divmod(t, wt)
        lt = jnp.sum(l, axis=0, keepdims=True)
        buf[row0 + r, :, c * LANE:(c + 1) * LANE] = (acc * (1.0 / lt)).astype(buf.dtype)

    def eloc(t):
        g, u = divmod(t, tpg)
        return sr[g % NBE], (g // NBE) * SK, u * LANE

    def pool_events(p, pos0, gap_, dly_, prow=None):
        kpt = LANE // WIN
        jj = jax.lax.broadcasted_iota(jnp.int32, (kpt, LANE), 0)
        ww = jax.lax.broadcasted_iota(jnp.int32, (kpt, LANE), 1)
        pool = jnp.where((ww >= jj * WIN) & (ww < (jj + 1) * WIN), 1.0 / (WIN * WIN), 0.0).astype(bf16)
        prow = p if prow is None else prow
        means = {}

        def piece(k):
            def run():
                i, c = divmod(k, wt)
                blk = x_vm[pl.ds(prow * rpp + i * WIN, WIN), :, c * LANE:(c + 1) * LANE]
                ssum = jnp.sum(blk.astype(f32), axis=0)
                hi = ssum.astype(bf16)
                lo = (ssum - hi.astype(f32)).astype(bf16)
                r = jax.lax.dot_general(pool, hi, NT, preferred_element_type=f32)
                r = jax.lax.dot_general(pool, lo, NT, preferred_element_type=f32) + r
                means[k] = r.astype(bf16)
            return run

        def proj():
            xs = jnp.concatenate([means[k] for k in range(2 * wt)], axis=0)
            xs_ref[prow] = pltpu.bitcast(xs, u32)
            at = jnp.dot(xs, pltpu.bitcast(wf_ref[0], bf16), preferred_element_type=f32)
            at_ref[p] = pltpu.bitcast(at.astype(bf16), u32)

        ev = [(pos0 + k * gap_, 0, piece(k)) for k in range(2 * wt)]
        ev.append((pos0 + (2 * wt - 1) * gap_ + dly_, 1, proj))
        return ev

    def proj_b(s):
        xs = jnp.concatenate([xs_ref[s * npair + q] for q in range(npair)], axis=0)
        bt = jax.lax.dot_general(pltpu.bitcast(wf_ref[1], bf16), pltpu.bitcast(xs, bf16), NT,
                                 preferred_element_type=f32)
        bt_ref[s] = pltpu.bitcast(bt.astype(bf16), u32)

    def qk_unit(t, p, q, n=1):
        def run():
            xt = jnp.concatenate([x_tile(0, t + i) for i in range(n)], axis=1)
            s = jnp.dot(pltpu.bitcast(at_ref[p], bf16), xt, preferred_element_type=f32)
            ref, r0, c0 = eloc(t)
            cols = slice(c0, c0 + n * LANE)
            if isinstance(q, int):
                ref[0, r0 + q * PK:r0 + (q + 1) * PK, cols] = s
            else:
                ref[0, pl.ds(pl.multiple_of(r0 + q * PK, 8), PK), cols] = s
            mp_ref[t // tpg, :, cols] = jnp.maximum(mp_ref[t // tpg, :, cols], _colmax(s))
        return run

    def pv_tile(t, s, zero):
        def run():
            never = zero != 0
            ref, r0, c0 = eloc(t)
            m_old = m_ref[t]
            m = _allmax(mp_ref[t // tpg, :, c0:c0 + LANE])
            m_ref[t] = m
            alpha = jnp.exp2(m_old - m)
            l, acc = _pv_block(ref[0, r0:r0 + SK, c0:c0 + LANE], m, zero, None, bt_ref[s], never)
            alpha = jnp.where(never, acc[0:8, :], alpha)
            acc_ref[t] = acc + (acc_ref[t].reshape(C // 8, 8, LANE) * alpha[None]).reshape(C, LANE)
            l_ref[t] = l + l_ref[t] * alpha
        return run

    @pl.when(step == 0)
    def _early():
        wcp = [pltpu.make_async_copy(a, b, wsem.at[0])
               for a, b in ((wq_hbm, wq_ref), (wkv_hbm, wkv_ref), (wo_hbm, wo_ref))]
        for c_ in wcp:
            c_.start()
        xcopy(0).start()
        for c_ in wcp:
            c_.wait()
        for p in range(1, NS * npair):
            xcopy(p).start()
        zi_ref[0] = 0
        for s_ in sr:
            s_[0, NK:NK + 8, :] = jnp.zeros((8, TQ), f32)

        def init(i, c):
            ts = pl.ds(i * tpg, tpg)
            m_ref[ts] = jnp.full((tpg, 8, LANE), -jnp.inf, f32)
            mp_ref[i] = jnp.full((8, TQ), -jnp.inf, f32)
            l_ref[ts] = jnp.zeros((tpg, 8, LANE), f32)
            acc_ref[ts] = jnp.zeros((tpg, C, LANE), f32)
            return c
        jax.lax.fori_loop(0, nte // tpg, init, 0)

        wa = jax.lax.dot_general(wkv_ref[:, :C], wq_ref[...], NT, preferred_element_type=f32)
        wa = wa * (C ** -0.5 * math.log2(math.e))
        wb = jnp.dot(wkv_ref[:, C:], wo_ref[...], preferred_element_type=f32)
        wf_ref[0] = pltpu.bitcast(wa.astype(bf16), u32)
        wf_ref[1] = pltpu.bitcast(wb.T.astype(bf16), u32)
        wf_ref[2] = pltpu.bitcast(wa.T.astype(bf16), u32)
        xcopy(0).wait()
        _interleave([], pool_events(0, 0, 0, 0))
        att_ref[...] = jnp.zeros(att_ref.shape, f32)
        att_ref[:, :PK] = jax.lax.dot_general(pltpu.bitcast(wf_ref[2], bf16), pltpu.bitcast(xs_ref[0], bf16), NT,
                                              preferred_element_type=f32)

        def table(it):
            def run():
                i = jnp.minimum(it, NVMAX // 4 - 1)
                v = pltpu.roll(att_ref[...], (LANE - (i // 2) * 8 - i % 2) % LANE, 1)
                for n, k in enumerate((0, 4, 2, 6)):
                    ab_ref[i * 4 + n] = jnp.broadcast_to(v[:, k:k + 1], (C, LANE)).reshape(C // 8, 8, LANE)
            return run

        def stage(s, carry):
            def quarter(q, c):
                p = s * npair + q
                xcopy(p + 1).wait()
                _interleave([qk_unit(t, p, q, tpg) for t in range(0, nte - late, tpg)],
                            pool_events(p + 1, off, gap, dly1) + [(0, 3, table(s * (npair - 1) + q))])
                return c
            jax.lax.fori_loop(0, npair - 1, quarter, 0)

            @pl.when(s + 1 < NS)
            def _():
                xcopy((s + 1) * npair).wait()
            nxt = jnp.minimum(s + 1, NS - 1) * npair
            q = npair - 1
            units = [(-2 if t < skew_e else t - skew_e, 0, qk_unit(t, s * npair + q, q))
                     for t in range(nte)]
            units += [(-1, qq * nte + t, qk_unit(t, s * npair + qq, qq))
                      for qq in range(q) for t in range(nte - late, nte)]
            zero = opaque_zero(NBE)
            units += [(t, 1, pv_tile(t, s, zero)) for t in range(nte)]
            units.sort(key=lambda e: e[:2])
            extra = pool_events(s * npair + npair, off2, gap2, dly, prow=nxt)
            _interleave([u[2] for u in units], extra + [(pb_pos, 2, lambda: proj_b(s))])
            return carry
        jax.lax.fori_loop(0, NS, stage, 0)

    @pl.when(step >= 1)
    def _main():
        row0 = RE + (step - 1) * R
        ntile = R * wt
        G = ntile // tpg
        nv = [NVMAX - 16 * (g < nsmall) for g in range(G)]
        zero = opaque_zero(G)
        never = zero != 0
        mx, vm, xq = {}, {}, {}
        last = step == pl.num_programs(0) - 1

        def at_rows(a, b):
            parts = []
            while a < b:
                p, o = divmod(a, PK)
                e = min(b - a, PK - o)
                parts.append(at_ref[p, o // 2:(o + e) // 2, :])
                a += e
            return parts[0] if len(parts) == 1 else jnp.concatenate(parts, axis=0)

        def bt_cols(a, b):
            parts = []
            while a < b:
                s_, o = divmod(a, SK)
                e = min(b - a, SK - o)
                parts.append(bt_ref[s_, :, o:o + e])
                a += e
            return parts[0] if len(parts) == 1 else jnp.concatenate(parts, axis=1)

        def early_out(t):
            k = step - 1
            src = jnp.minimum(k, nev - 1) * (NR * wt) + t
            normalise(oe_vm, jnp.minimum(k, nev) * NR, t, acc_ref[src], l_ref[src])

        slots = []
        for g in range(G):
            nm = NK - nv[g]
            lo, hi = (0 if g == 0 else t0), nm - (t1 if g < G - 1 else tl)
            slots += [(g, r, 0.0 if r < lo or r > hi else f1 if g < G - 1 and r >= nm - w1 else 1.0)
                      for r in range(0, nm, 16)]
        room, todo = sum(e[2] for e in slots), sum(nv) * tpg // 2
        used, cum = set(), 0.0
        for g, r, w in slots:
            cum += w
            if len(used) < todo and (len(used) + 1) * room / todo <= cum + 1e-9:
                used.add((g, r))
        assert len(used) == todo
        queue = []

        def markers(n):
            parts = []
            while n:
                if not queue:
                    t = len(vm)
                    g, u = divmod(t, tpg)
                    us = slice(u * LANE, (u + 1) * LANE)
                    sv, mk = _vpu_scores(xq[g][:, us] if g in xq else x_tile(row0, t), ab_ref[0:nv[g]])
                    sr[g][0, 0:nv[g], us] = sv.reshape(nv[g], LANE)
                    vm[t] = jnp.max(sv, axis=0)
                    queue.append(mk)
                mk = queue.pop()
                parts.append(mk[:n])
                if mk.shape[0] > n:
                    queue.append(mk[n:])
                n -= parts[-1].shape[0]
            return parts[0] if len(parts) == 1 else jnp.concatenate(parts, axis=0)

        for g in range(G):
            xq[g] = jnp.concatenate([x_tile(row0, g * tpg + t) for t in range(tpg)], axis=1)
            for a in range(nv[g], NK, LANE):
                b = min(a + LANE, NK)
                s = jnp.dot(pltpu.bitcast(at_rows(a, b), bf16), xq[g], preferred_element_type=f32)
                flags = [(g, r - nv[g]) in used for r in range(a, b, 16)]
                if any(flags):
                    s0 = s[:, :LANE].reshape((b - a) // 16, 2, 8, LANE)
                    parts, i = [], 0
                    for f, run in itertools.groupby(flags):
                        n = len(list(run))
                        v = s0[i:i + n, 0]
                        parts.append(jnp.where(never, markers(n), v) if f else v)
                        i += n
                    s0 = jnp.stack([jnp.concatenate(parts, axis=0), s0[:, 1]], axis=1)
                    s = jnp.concatenate([s0.reshape(b - a, LANE), s[:, LANE:]], axis=1)
                sr[g][0, a:b, :] = s
                mx[g] = jnp.maximum(mx[g], _colmax(s)) if g in mx else _colmax(s)
            if g < NR * wt:
                early_out(g)

        for t in range(ntile):
            g, u = divmod(t, tpg)
            us = slice(u * LANE, (u + 1) * LANE)
            m = _allmax(jnp.maximum(vm[t], mx[g][:, us]))
            l, acc = zero, None
            for j in range(NK // KP):
                l, acc = _pv_block(sr[g][0, j * KP:(j + 1) * KP, us], m, l, acc,
                                   bt_cols(j * KP, (j + 1) * KP), never)
            normalise(x_vm, row0, t, acc, l)
            if t + 1 == (R - RO) * wt:
                pl.when(last)(lambda: ocopy(x_vm, H - R, R - RO).start())
        pl.when(jnp.logical_not(last))(lambda: ocopy(x_vm, row0, R).start())

    @pl.when(step == nev)
    def _():
        ocopy(oe_vm, 0, RE).start()

    @pl.when(step == pl.num_programs(0) - 1)
    def _():
        ocopy(x_vm, H - RO, RO).start()
        ocopy(x_vm, 0, H).wait()


@jax.jit
def pallas_standalone__window_attn_twins__vision_kernel(x, wq, wkv, wo):
    B, H, W, C = x.shape
    nk = (H // WIN) * (W // WIN)
    pk = 2 * W // WIN
    nte = RE * W // LANE
    nsteps = (H - RE) // R
    assert B == 1 and nk % SK == 0 and SK % pk == 0 and W % LANE == 0 and C % 16 == 0
    assert (H - RE) % R == 0 and RE <= 4 * WIN and nsteps >= RE // NR
    xt = jnp.transpose(x, (0, 1, 3, 2)).reshape(H, C, W)
    out = pl.pallas_call(
        functools.partial(_kernel, H=H, W=W, C=C, **CFG),
        grid=(1 + nsteps,),
        in_specs=[pl.BlockSpec(memory_space=pl.ANY)] * 4,
        out_specs=pl.BlockSpec(memory_space=pl.ANY),
        out_shape=jax.ShapeDtypeStruct((H, C, W), x.dtype),
        scratch_shapes=[
            pltpu.VMEM((RE + NR, C, W), bf16), pltpu.SemaphoreType.DMA((1,)),
            pltpu.VMEM((H, C, W), bf16), pltpu.SemaphoreType.DMA((nk // pk,)),
            pltpu.VMEM((C, C), bf16), pltpu.VMEM((C, 2 * C), bf16), pltpu.VMEM((C, C), bf16),
            pltpu.SemaphoreType.DMA((1,)),
            pltpu.VMEM((nk // pk + 1, pk // 2, C), u32),
            pltpu.VMEM((nk // SK, C // 2, SK), u32),
            pltpu.VMEM((3, C // 2, C), u32),
            pltpu.VMEM((nk // pk, pk // 2, C), u32),
            pltpu.SMEM((1,), jnp.int32),
            pltpu.VMEM((nte * LANE // TQ, 8, TQ), f32), pltpu.VMEM((nte, 8, LANE), f32),
            pltpu.VMEM((nte, 8, LANE), f32), pltpu.VMEM((nte, C, LANE), f32),
            pltpu.VMEM((C, LANE), f32), pltpu.VMEM((NVMAX, C // 8, 8, LANE), f32),
        ] + [pltpu.VMEM((1, nk + 8, TQ), f32)] * (R * W // TQ),
        compiler_params=pltpu.CompilerParams(
            dimension_semantics=("arbitrary",),
            vmem_limit_bytes=110 * 1024 * 1024,
        ),
    )(xt, wq, wkv, wo)
    return jnp.transpose(out.reshape(1, H, C, W), (0, 1, 3, 2))
```

```python
import functools
import itertools
import math

import jax
import jax.numpy as jnp
import jax.experimental.pallas as pl
import jax.experimental.pallas.tpu as pltpu

f32, bf16, u32 = jnp.float32, jnp.bfloat16, jnp.uint32
WIN = 8
LANE = 128
NT = (((1,), (1,)), ((), ()))

R = 16
RE = 32
SK = 384
TQ = 512
KP = 256
NR = 2
CUTS = (0, 12, 15, 16)
NVMAX = 64
CFG = dict(nsmall=2, t0=64, t1=8, tl=400, w1=250, f1=0.7,
           gap=3, off=2, dly1=2, dly=8, gap2=4, skew_e=6, off2=6, pb_pos=10, late=8)


def _colmax(s):
    return jnp.max(s.reshape(s.shape[0] // 8, 8, s.shape[1]), axis=0)


def _allmax(m):
    return jnp.broadcast_to(jnp.max(m, axis=0, keepdims=True), m.shape)


def _pv_block(sv, m, l, acc, bt, never):
    nk = sv.shape[0]
    p = jnp.exp2(sv.reshape(nk // LANE, LANE // 8, 8, LANE) - m[None, None])
    ps = jnp.sum(p, axis=1)
    parts = []
    for k in range(nk // LANE):
        l = l + ps[k]
        parts += [jnp.where(never, l, p[k, 0])[None], p[k, 1:]]
    p = jnp.concatenate(parts, axis=0).reshape(nk, LANE)
    o = jnp.dot(pltpu.bitcast(bt, bf16), p.astype(bf16), preferred_element_type=f32)
    return l, (o if acc is None else o + acc)


def _merge(a, b, s):
    ax = a.ndim - 2
    low = (jax.lax.broadcasted_iota(jnp.int32, a.shape, ax) & s) == 0
    if s == 4:
        return jnp.where(low, a, b) + pltpu.roll(jnp.where(low, b, a), 4, ax)
    return jnp.where(low, a + pltpu.roll(a, 8 - s, ax), b + pltpu.roll(b, s, ax))


def _vpu_scores(xt, ab):
    n = ab.shape[0] // 8
    xf = xt.astype(f32).reshape(1, xt.shape[0] // 8, 8, LANE)
    h = jnp.sum(ab * xf, axis=1).reshape(n * 4, 2, 8, LANE)
    p = _merge(h[:, 0], h[:, 1], 4).reshape(n * 2, 2, 8, LANE)
    q = _merge(p[:, 0], p[:, 1], 2).reshape(n, 2, 8, LANE)
    f = _merge(q[:, 0], q[:, 1], 1)
    pe = p[:, 0].reshape(n, 2, 8, LANE)
    return f, jnp.stack([pe[:, 0], q[:, 0], pe[:, 1], f], axis=1).reshape(n * 4, 8, LANE)


def _interleave(main, extra):
    extra = sorted(extra, key=lambda e: e[:2])
    for i, fn in enumerate(main):
        while extra and extra[0][0] <= i:
            extra.pop(0)[2]()
        fn()
    for e in extra:
        e[2]()


def _kernel(x_hbm, wq_hbm, wkv_hbm, wo_hbm, o_hbm,
            oe_vm, osem, x_vm, xsems, wq_ref, wkv_ref, wo_ref, wsem, at_ref, bt_ref, wf_ref, xs_ref,
            zi_ref, mp_ref, m_ref, l_ref, acc_ref, att_ref, ab_ref, *sr,
            H, W, C, nsmall, t0, t1, tl, w1, f1, gap, off, dly, gap2, skew_e, off2, pb_pos, late, dly1):
    step = pl.program_id(0)
    NS = bt_ref.shape[0]
    NK = NS * SK
    PK = 2 * W // WIN
    rpp = 2 * WIN
    npair = SK // PK
    wt = W // LANE
    tpg = TQ // LANE
    nte = RE * wt
    nev = RE // NR
    NBE = -(-nte // (NS * tpg))

    def xcopy(p):
        rows = pl.ds(p * rpp, rpp)
        return pltpu.make_async_copy(x_hbm.at[rows], x_vm.at[rows], xsems.at[p])

    def ocopy(buf, r0, n):
        rows = pl.ds(r0, n)
        return pltpu.make_async_copy(buf.at[rows], o_hbm.at[rows], osem.at[0])

    def opaque_zero(n):
        zd = zi_ref[0]
        return sum(s_[zd, NK:NK + 8, 0:LANE] for s_ in sr[:n])

    def x_tile(row0, t):
        return x_vm[row0 + t // wt, :, (t % wt) * LANE:(t % wt + 1) * LANE]

    def normalise(buf, row0, t, acc, l):
        r, c = divmod(t, wt)
        lt = jnp.sum(l, axis=0, keepdims=True)
        buf[row0 + r, :, c * LANE:(c + 1) * LANE] = (acc * (1.0 / lt)).astype(buf.dtype)

    def eloc(t):
        g, u = divmod(t, tpg)
        return sr[g % NBE], (g // NBE) * SK, u * LANE

    def pool_events(p, pos0, gap_, dly_, prow=None):
        kpt = LANE // WIN
        jj = jax.lax.broadcasted_iota(jnp.int32, (kpt, LANE), 0)
        ww = jax.lax.broadcasted_iota(jnp.int32, (kpt, LANE), 1)
        pool = jnp.where((ww >= jj * WIN) & (ww < (jj + 1) * WIN), 1.0 / (WIN * WIN), 0.0).astype(bf16)
        prow = p if prow is None else prow
        means = {}

        def piece(k):
            def run():
                i, c = divmod(k, wt)
                blk = x_vm[pl.ds(prow * rpp + i * WIN, WIN), :, c * LANE:(c + 1) * LANE]
                ssum = jnp.sum(blk.astype(f32), axis=0)
                hi = ssum.astype(bf16)
                lo = (ssum - hi.astype(f32)).astype(bf16)
                r = jax.lax.dot_general(pool, hi, NT, preferred_element_type=f32)
                r = jax.lax.dot_general(pool, lo, NT, preferred_element_type=f32) + r
                means[k] = r.astype(bf16)
            return run

        def proj():
            xs = jnp.concatenate([means[k] for k in range(2 * wt)], axis=0)
            xs_ref[prow] = pltpu.bitcast(xs, u32)
            at = jnp.dot(xs, pltpu.bitcast(wf_ref[0], bf16), preferred_element_type=f32)
            at_ref[p] = pltpu.bitcast(at.astype(bf16), u32)

        ev = [(pos0 + k * gap_, 0, piece(k)) for k in range(2 * wt)]
        ev.append((pos0 + (2 * wt - 1) * gap_ + dly_, 1, proj))
        return ev

    def fresh(v, zero):
        z = pltpu.bitcast(zero, u32)
        z = jnp.concatenate([z] * -(-v.shape[1] // LANE), axis=1)[:, :v.shape[1]]
        return (v.reshape(v.shape[0] // 8, 8, v.shape[1]) | z[None]).reshape(v.shape)

    def proj_b(s, cur, zero):
        xs = jnp.concatenate([xs_ref[s * npair + q] for q in range(npair)], axis=0)
        bt = jax.lax.dot_general(pltpu.bitcast(wf_ref[1], bf16), pltpu.bitcast(xs, bf16), NT,
                                 preferred_element_type=f32)
        bt_ref[s] = pltpu.bitcast(bt.astype(bf16), u32)
        cur.append(fresh(pltpu.bitcast(bt.astype(bf16), u32), zero))

    def qk_unit(t, at, q, n=1):
        def run():
            xt = jnp.concatenate([x_tile(0, t + i) for i in range(n)], axis=1)
            s = jnp.dot(pltpu.bitcast(at, bf16), xt, preferred_element_type=f32)
            ref, r0, c0 = eloc(t)
            cols = slice(c0, c0 + n * LANE)
            if isinstance(q, int):
                ref[0, r0 + q * PK:r0 + (q + 1) * PK, cols] = s
            else:
                ref[0, pl.ds(pl.multiple_of(r0 + q * PK, 8), PK), cols] = s
            mp_ref[t // tpg, :, cols] = jnp.maximum(mp_ref[t // tpg, :, cols], _colmax(s))
        return run

    def pv_tile(t, cur, zero):
        def run():
            never = zero != 0
            ref, r0, c0 = eloc(t)
            m_old = m_ref[t]
            m = _allmax(mp_ref[t // tpg, :, c0:c0 + LANE])
            m_ref[t] = m
            alpha = jnp.exp2(m_old - m)
            l, acc = _pv_block(ref[0, r0:r0 + SK, c0:c0 + LANE], m, zero, None, cur[0], never)
            alpha = jnp.where(never, acc[0:8, :], alpha)
            acc_ref[t] = acc + (acc_ref[t].reshape(C // 8, 8, LANE) * alpha[None]).reshape(C, LANE)
            l_ref[t] = l + l_ref[t] * alpha
        return run

    @pl.when(step == 0)
    def _early():
        wcp = [pltpu.make_async_copy(a, b, wsem.at[0])
               for a, b in ((wq_hbm, wq_ref), (wkv_hbm, wkv_ref), (wo_hbm, wo_ref))]
        for c_ in wcp:
            c_.start()
        xcopy(0).start()
        for c_ in wcp:
            c_.wait()
        for p in range(1, NS * npair):
            xcopy(p).start()
        zi_ref[0] = 0
        for s_ in sr:
            s_[0, NK:NK + 8, :] = jnp.zeros((8, TQ), f32)

        def init(i, c):
            ts = pl.ds(i * tpg, tpg)
            m_ref[ts] = jnp.full((tpg, 8, LANE), -jnp.inf, f32)
            mp_ref[i] = jnp.full((8, TQ), -jnp.inf, f32)
            l_ref[ts] = jnp.zeros((tpg, 8, LANE), f32)
            acc_ref[ts] = jnp.zeros((tpg, C, LANE), f32)
            return c
        jax.lax.fori_loop(0, nte // tpg, init, 0)

        wa = jax.lax.dot_general(wkv_ref[:, :C], wq_ref[...], NT, preferred_element_type=f32)
        wa = wa * (C ** -0.5 * math.log2(math.e))
        wb = jnp.dot(wkv_ref[:, C:], wo_ref[...], preferred_element_type=f32)
        wf_ref[0] = pltpu.bitcast(wa.astype(bf16), u32)
        wf_ref[1] = pltpu.bitcast(wb.T.astype(bf16), u32)
        wf_ref[2] = pltpu.bitcast(wa.T.astype(bf16), u32)
        xcopy(0).wait()
        _interleave([], pool_events(0, 0, 0, 0))
        att_ref[...] = jnp.zeros(att_ref.shape, f32)
        att_ref[:, :PK] = jax.lax.dot_general(pltpu.bitcast(wf_ref[2], bf16), pltpu.bitcast(xs_ref[0], bf16), NT,
                                              preferred_element_type=f32)

        def table(it):
            def run():
                i = jnp.minimum(it, NVMAX // 4 - 1)
                v = pltpu.roll(att_ref[...], (LANE - (i // 2) * 8 - i % 2) % LANE, 1)
                for n, k in enumerate((0, 4, 2, 6)):
                    ab_ref[i * 4 + n] = jnp.broadcast_to(v[:, k:k + 1], (C, LANE)).reshape(C // 8, 8, LANE)
            return run

        def stage(s, carry):
            def quarter(q, c):
                p = s * npair + q
                xcopy(p + 1).wait()
                at = at_ref[p]
                _interleave([qk_unit(t, at, q, tpg) for t in range(0, nte - late, tpg)],
                            pool_events(p + 1, off, gap, dly1) + [(0, 3, table(s * (npair - 1) + q))])
                return c
            jax.lax.fori_loop(0, npair - 1, quarter, 0)

            @pl.when(s + 1 < NS)
            def _():
                xcopy((s + 1) * npair).wait()
            nxt = jnp.minimum(s + 1, NS - 1) * npair
            q = npair - 1
            zero = opaque_zero(NBE)
            ats = [at_ref[s * npair + qq] for qq in range(npair)]
            at = fresh(ats[q], zero)
            units = [(-2, 0, qk_unit(t, ats[q], q)) if t < skew_e else (t - skew_e, 0, qk_unit(t, at, q))
                     for t in range(nte)]
            units += [(-1, qq * nte + t, qk_unit(t, ats[qq], qq))
                      for qq in range(q) for t in range(nte - late, nte)]
            cur = []
            units += [(t, 1, pv_tile(t, cur, zero)) for t in range(nte)]
            units.sort(key=lambda e: e[:2])
            extra = pool_events(s * npair + npair, off2, gap2, dly, prow=nxt)
            _interleave([u[2] for u in units], extra + [(pb_pos, 2, lambda: proj_b(s, cur, zero))])
            return carry
        jax.lax.fori_loop(0, NS, stage, 0)

    @pl.when(step >= 1)
    def _main():
        row0 = RE + (step - 1) * R
        ntile = R * wt
        G = ntile // tpg
        nv = [NVMAX - 16 * (g < nsmall) for g in range(G)]
        zero = opaque_zero(G)
        never = zero != 0
        mx, vm, xq = {}, {}, {}
        last = step == pl.num_programs(0) - 1

        def at_rows(a, b):
            parts = []
            while a < b:
                p, o = divmod(a, PK)
                e = min(b - a, PK - o)
                parts.append(at_ref[p, o // 2:(o + e) // 2, :])
                a += e
            return parts[0] if len(parts) == 1 else jnp.concatenate(parts, axis=0)

        def bt_cols(a, b):
            parts = []
            while a < b:
                s_, o = divmod(a, SK)
                e = min(b - a, SK - o)
                parts.append(bt_ref[s_, :, o:o + e])
                a += e
            return parts[0] if len(parts) == 1 else jnp.concatenate(parts, axis=1)

        def early_out(t):
            k = step - 1
            src = jnp.minimum(k, nev - 1) * (NR * wt) + t
            normalise(oe_vm, jnp.minimum(k, nev) * NR, t, acc_ref[src], l_ref[src])

        slots = []
        for g in range(G):
            nm = NK - nv[g]
            lo, hi = (0 if g == 0 else t0), nm - (t1 if g < G - 1 else tl)
            slots += [(g, r, 0.0 if r < lo or r > hi else f1 if g < G - 1 and r >= nm - w1 else 1.0)
                      for r in range(0, nm, 16)]
        room, todo = sum(e[2] for e in slots), sum(nv) * tpg // 2
        used, cum = set(), 0.0
        for g, r, w in slots:
            cum += w
            if len(used) < todo and (len(used) + 1) * room / todo <= cum + 1e-9:
                used.add((g, r))
        assert len(used) == todo
        queue = []

        def markers(n):
            parts = []
            while n:
                if not queue:
                    t = len(vm)
                    g, u = divmod(t, tpg)
                    us = slice(u * LANE, (u + 1) * LANE)
                    sv, mk = _vpu_scores(xq[g][:, us] if g in xq else x_tile(row0, t), ab_ref[0:nv[g]])
                    sr[g][0, 0:nv[g], us] = sv.reshape(nv[g], LANE)
                    vm[t] = jnp.max(sv, axis=0)
                    queue.append(mk)
                mk = queue.pop()
                parts.append(mk[:n])
                if mk.shape[0] > n:
                    queue.append(mk[n:])
                n -= parts[-1].shape[0]
            return parts[0] if len(parts) == 1 else jnp.concatenate(parts, axis=0)

        for g in range(G):
            xq[g] = jnp.concatenate([x_tile(row0, g * tpg + t) for t in range(tpg)], axis=1)
            for a in range(nv[g], NK, LANE):
                b = min(a + LANE, NK)
                s = jnp.dot(pltpu.bitcast(at_rows(a, b), bf16), xq[g], preferred_element_type=f32)
                flags = [(g, r - nv[g]) in used for r in range(a, b, 16)]
                if any(flags):
                    s0 = s[:, :LANE].reshape((b - a) // 16, 2, 8, LANE)
                    parts, i = [], 0
                    for f, run in itertools.groupby(flags):
                        n = len(list(run))
                        v = s0[i:i + n, 0]
                        parts.append(jnp.where(never, markers(n), v) if f else v)
                        i += n
                    s0 = jnp.stack([jnp.concatenate(parts, axis=0), s0[:, 1]], axis=1)
                    s = jnp.concatenate([s0.reshape(b - a, LANE), s[:, LANE:]], axis=1)
                sr[g][0, a:b, :] = s
                mx[g] = jnp.maximum(mx[g], _colmax(s)) if g in mx else _colmax(s)
            if g < NR * wt:
                early_out(g)

        for t in range(ntile):
            g, u = divmod(t, tpg)
            us = slice(u * LANE, (u + 1) * LANE)
            m = _allmax(jnp.maximum(vm[t], mx[g][:, us]))
            l, acc = zero, None
            for j in range(NK // KP):
                l, acc = _pv_block(sr[g][0, j * KP:(j + 1) * KP, us], m, l, acc,
                                   bt_cols(j * KP, (j + 1) * KP), never)
            normalise(x_vm, row0, t, acc, l)
            for a, b in zip(CUTS[:-2], CUTS[1:-1]):
                if t + 1 == b * wt:
                    pl.when(last)(lambda: ocopy(x_vm, H - R + a, b - a).start())
        pl.when(jnp.logical_not(last))(lambda: ocopy(x_vm, row0, R).start())

    @pl.when(step == nev)
    def _():
        ocopy(oe_vm, 0, RE).start()

    @pl.when(step == pl.num_programs(0) - 1)
    def _():
        ocopy(x_vm, H - R + CUTS[-2], R - CUTS[-2]).start()
        ocopy(x_vm, 0, H).wait()


@jax.jit
def pallas_standalone__window_attn_twins__vision_kernel(x, wq, wkv, wo):
    B, H, W, C = x.shape
    nk = (H // WIN) * (W // WIN)
    pk = 2 * W // WIN
    nte = RE * W // LANE
    nsteps = (H - RE) // R
    assert B == 1 and nk % SK == 0 and SK % pk == 0 and W % LANE == 0 and C % 16 == 0
    assert (H - RE) % R == 0 and RE <= 4 * WIN and nsteps >= RE // NR
    assert NVMAX <= pk <= LANE and (nk // SK) * (SK // pk - 1) >= NVMAX // 4 and RE * SK <= R * nk
    xt = jnp.transpose(x, (0, 1, 3, 2)).reshape(H, C, W)
    out = pl.pallas_call(
        functools.partial(_kernel, H=H, W=W, C=C, **CFG),
        grid=(1 + nsteps,),
        in_specs=[pl.BlockSpec(memory_space=pl.ANY)] * 4,
        out_specs=pl.BlockSpec(memory_space=pl.ANY),
        out_shape=jax.ShapeDtypeStruct((H, C, W), x.dtype),
        scratch_shapes=[
            pltpu.VMEM((RE + NR, C, W), bf16), pltpu.SemaphoreType.DMA((1,)),
            pltpu.VMEM((H, C, W), bf16), pltpu.SemaphoreType.DMA((nk // pk,)),
            pltpu.VMEM((C, C), bf16), pltpu.VMEM((C, 2 * C), bf16), pltpu.VMEM((C, C), bf16),
            pltpu.SemaphoreType.DMA((1,)),
            pltpu.VMEM((nk // pk + 1, pk // 2, C), u32),
            pltpu.VMEM((nk // SK, C // 2, SK), u32),
            pltpu.VMEM((3, C // 2, C), u32),
            pltpu.VMEM((nk // pk, pk // 2, C), u32),
            pltpu.SMEM((1,), jnp.int32),
            pltpu.VMEM((nte * LANE // TQ, 8, TQ), f32), pltpu.VMEM((nte, 8, LANE), f32),
            pltpu.VMEM((nte, 8, LANE), f32), pltpu.VMEM((nte, C, LANE), f32),
            pltpu.VMEM((C, LANE), f32), pltpu.VMEM((NVMAX, C // 8, 8, LANE), f32),
        ] + [pltpu.VMEM((1, nk + 8, TQ), f32)] * (R * W // TQ),
        compiler_params=pltpu.CompilerParams(
            dimension_semantics=("arbitrary",),
            vmem_limit_bytes=110 * 1024 * 1024,
        ),
    )(xt, wq, wkv, wo)
    return jnp.transpose(out.reshape(1, H, C, W), (0, 1, 3, 2))
```
